```python
import jax
import jax.numpy as jnp

def _softmax(x, axis=-1):
    return jax.nn.softmax(x, axis=axis)
def _gelu(x):
    return jax.nn.gelu(x, approximate=True)
def _silu(x):
    return jax.nn.silu(x)
def _sigmoid(x):
    return jax.nn.sigmoid(x)
def _layernorm(x, axis=-1, eps=1e-5):
    m = jnp.mean(x, axis=axis, keepdims=True)
    v = jnp.var(x, axis=axis, keepdims=True)
    return (x - m) / jnp.sqrt(v + eps)
def _scatter_add(tgt, idx, src, axis=0):
    return tgt.at[idx].add(src)
def _segment_sum(src, seg, n):
    return jax.ops.segment_sum(src, seg, n)
class _Rng:
    def __init__(self, key):
        self._k = key
    def _next(self):
        self._k, sub = jax.random.split(self._k)
        return sub
    def normal(self, shape):
        return jax.random.normal(self._next(), shape, dtype=jnp.bfloat16)
    def randint(self, lo, hi, shape):
        return jax.random.randint(self._next(), shape, lo, hi, dtype=jnp.int32)
    def uniform(self, shape, lo=0.0, hi=1.0):
        return jax.random.uniform(self._next(), shape, jnp.bfloat16, lo, hi)
    def permutation(self, n):
        return jax.random.permutation(self._next(), n)


kernel_name = 'interleave_layers__gqa_block_cached__sliding_block_cached__decode'

def _fwd_setup_inputs():
    _rng = _Rng(jax.random.key(int.from_bytes(__import__("os").urandom(4), "little")))
    _w = (lambda a: (lambda t: t.astype(jnp.bfloat16) if jnp.issubdtype(t.dtype, jnp.floating) else t)(jnp.asarray(a)))
    def _A_setup():
        B, Sq, D = 1, 1, 640
        Hq, Hkv, Sk, Dh = 32, 32, 8192, 128
        assert Hq % Hkv == 0, (Hq, Hkv)
        return {
            "x": _w((lambda *s: _rng.normal(s) * 0.05)(B, Sq, D)),
            "k_cache": _w((lambda *s: _rng.normal(s) * 0.05)(B, Hkv, Sk, Dh)),
            "v_cache": _w((lambda *s: _rng.normal(s) * 0.05)(B, Hkv, Sk, Dh)),
            "wq": _w((lambda *s: _rng.normal(s) * 0.05)(D, Hq * Dh) * (D ** -0.5)),
            "wo": _w((lambda *s: _rng.normal(s) * 0.05)(Hq * Dh, D) * ((Hq * Dh) ** -0.5)),
        }
    _A_in = _A_setup()

    def _B_setup():
        B, Sq, D = 1, 1, 640
        Hq, Hkv, Sk, Dh = 32, 32, 8192, 128
        assert Hq % Hkv == 0, (Hq, Hkv)
        return {
            "x": _w((lambda *s: _rng.normal(s) * 0.05)(B, Sq, D)),
            "k_cache": _w((lambda *s: _rng.normal(s) * 0.05)(B, Hkv, Sk, Dh)),
            "v_cache": _w((lambda *s: _rng.normal(s) * 0.05)(B, Hkv, Sk, Dh)),
            "wq": _w((lambda *s: _rng.normal(s) * 0.05)(D, Hq * Dh) * (D ** -0.5)),
            "wo": _w((lambda *s: _rng.normal(s) * 0.05)(Hq * Dh, D) * ((Hq * Dh) ** -0.5)),
        }
    _B_in = _B_setup()

    return {
        "A_x": _A_in["x"],
        "A_k_cache": _A_in["k_cache"],
        "A_v_cache": _A_in["v_cache"],
        "A_wq": _A_in["wq"],
        "A_wo": _A_in["wo"],
        "B_x": _B_in["x"],
        "B_k_cache": _B_in["k_cache"],
        "B_v_cache": _B_in["v_cache"],
        "B_wq": _B_in["wq"],
        "B_wo": _B_in["wo"],
    }

def _fwd_reference(A_x, A_k_cache, A_v_cache, A_wq, A_wo, B_x, B_k_cache, B_v_cache, B_wq, B_wo):
    def _A_ref(x, k_cache, v_cache, wq, wo):
        B, Sq, D = x.shape
        Hq, Dh = 32, 128
        Hkv = k_cache.shape[1]
        rep = Hq // Hkv
        q = (lambda x, *d: x.transpose(*d))((x @ wq).reshape(B, Sq, Hq, Dh), 0, 2, 1, 3)
        k = jnp.repeat(k_cache, rep, axis=1)
        v = jnp.repeat(v_cache, rep, axis=1)
        scores = jnp.einsum("bhqd,bhkd->bhqk", q, k) * (Dh ** -0.5)
        p = _softmax(scores, axis=-1)
        o = jnp.einsum("bhqk,bhkd->bhqd", p, v)
        return (lambda x, *d: x.transpose(*d))(o, 0, 2, 1, 3).reshape(B, Sq, Hq * Dh) @ wo

    def _B_ref(x, k_cache, v_cache, wq, wo):
        B, Sq, D = x.shape
        Hq, Dh = 32, 128
        Hkv, Sk = k_cache.shape[1], k_cache.shape[2]
        W = min(4096, max(256, Sk // 4))
        rep = Hq // Hkv
        q = (lambda x, *d: x.transpose(*d))((x @ wq).reshape(B, Sq, Hq, Dh), 0, 2, 1, 3)
        k = jnp.repeat(k_cache[:, :, Sk - W:, :], rep, axis=1)
        v = jnp.repeat(v_cache[:, :, Sk - W:, :], rep, axis=1)
        scores = jnp.einsum("bhqd,bhkd->bhqk", q, k) * (Dh ** -0.5)
        p = _softmax(scores, axis=-1)
        o = jnp.einsum("bhqk,bhkd->bhqd", p, v)
        return (lambda x, *d: x.transpose(*d))(o, 0, 2, 1, 3).reshape(B, Sq, Hq * Dh) @ wo

    x = A_x
    x = x + _A_ref(_layernorm(x, axis=-1), A_k_cache, A_v_cache, A_wq, A_wo)
    x = x + _B_ref(_layernorm(x, axis=-1), B_k_cache, B_v_cache, B_wq, B_wo)
    x = x + _A_ref(_layernorm(x, axis=-1), A_k_cache, A_v_cache, A_wq, A_wo)
    x = x + _B_ref(_layernorm(x, axis=-1), B_k_cache, B_v_cache, B_wq, B_wo)
    return x


def setup_inputs():
    _inp = _fwd_setup_inputs()
    _gk = jax.random.fold_in(jax.random.key(int.from_bytes(__import__("os").urandom(4), "little")), 2**31 - 1)
    _shapes = [[1, 1, 640]]
    _dtypes = ['bfloat16']
    _gks = jax.random.split(_gk, len(_shapes))
    _gs = [jax.random.normal(k, s, dtype=jnp.dtype(d)) * 0.05 for k, s, d in zip(_gks, _shapes, _dtypes)]
    _inp["grad_out"] = _gs[0]
    return _inp

def reference(A_x, A_k_cache, A_v_cache, A_wq, A_wo, B_k_cache, B_v_cache, B_wq, B_wo, B_x, grad_out):
    _const = dict(B_x=B_x)
    def _f(*_d):
        return _fwd_reference(**{'A_x': _d[0], 'A_k_cache': _d[1], 'A_v_cache': _d[2], 'A_wq': _d[3], 'A_wo': _d[4], 'B_k_cache': _d[5], 'B_v_cache': _d[6], 'B_wq': _d[7], 'B_wo': _d[8], **_const})
    _out, _vjp = jax.vjp(_f, A_x, A_k_cache, A_v_cache, A_wq, A_wo, B_k_cache, B_v_cache, B_wq, B_wo)
    _grads = _vjp(grad_out)
    _out0 = jnp.asarray(_out)
    return (_out0, *[jnp.asarray(_g) for _g in _grads])
```

```python
import jax
import jax.numpy as jnp
from jax import lax
import jax.experimental.pallas as pl
import jax.experimental.pallas.tpu as pltpu

F32 = jnp.float32
BF16 = jnp.bfloat16

D = 640
H = 32
DH = 128
UNIT = 2048
T = 128
NT = UNIT // T
NG = H // 4
SCALE = DH ** -0.5
EPS = 1e-5

NSLOT = 12
NRES = NSLOT - 2
SPAN = 2
UNROLL3 = 16
ZSEG = 16

_NT_DIMS = (((1,), (1,)), ((), ()))
_TN_DIMS = (((0,), (0,)), ((), ()))


def _slot_plan():
    slot = list(range(NRES))
    kb_slot = [None] * NG
    kb_slot[NG - 2], kb_slot[NG - 1] = NRES, NRES + 1
    pm_slot = []
    refill = []
    todo = [("A", h) for h in range(NRES, H)] + [("B", g) for g in range(NG - 2)]
    for h in range(H):
        if h % 16 == 0:
            pm_slot.append(slot[h])
            refill.append(None)
        elif todo:
            kind, idx = todo.pop(0)
            refill.append((kind, idx))
            if kind == "A":
                slot.append(slot[h])
            else:
                kb_slot[idx] = slot[h]
        else:
            refill.append(None)
    spare = [s for s in range(NSLOT) if s not in pm_slot and s not in kb_slot]
    assert not todo and len(slot) == H and spare
    pb_slot = spare[0]
    stage = [s for s in range(NSLOT) if s not in pm_slot and s != pb_slot]
    return slot, kb_slot, pm_slot, refill, pb_slot, stage


A_SLOT, KB_SLOT, PM_SLOT, REFILL, PB_SLOT, STAGE_SLOT = _slot_plan()
NSTAGE = len(STAGE_SLOT) // 2
FIRST_B_REFILL = min(h for h in range(H) if REFILL[h] and REFILL[h][0] == "B")
LAST_REFILL = max(h for h in range(H) if REFILL[h])

NZERO = 2 * 3 * NT * (H // ZSEG)
READS_AFTER_HEAD = 6
NZERO_EARLY = 28

TAB_A, TAB_KB, TAB_STAGE = 0, H, H + NG
TAB_SIZE = H + NG + 2 * NSTAGE

V_H, V_G, V_INV = 0, 4, 8


MARKS = False
DEBUG = {}


class _Marks:
    def __init__(self):
        self.cur = None

    def __call__(self, name):
        if not MARKS:
            return
        if self.cur is not None:
            self.cur.__exit__(None, None, None)
            self.cur = None
        if name:
            self.cur = jax.named_scope("ph_" + name)
            self.cur.__enter__()


def _kernel(
    x_hbm, g_hbm, ka_hbm, va_hbm, wqa_hbm, woa_hbm, kb_hbm, vb_hbm, wqb_hbm, wob_hbm,
    out_hbm, dx_hbm, dka_hbm, dva_hbm, dwqa_hbm, dwoa_hbm, dkb_hbm, dvb_hbm, dwqb_hbm, dwob_hbm,
    va, vb, wqa, woa, wqb, wob, pool, m1, zeros, s_buf, p_cur,
    qa1, qa3, oa1, oa3, doa1, doa3, dqa1, dqa3, qb, ob, dob, dqb, vec,
    x_in, g_in, out_st, dx_st, tab,
    sem_a, sem_b, sem_slot, sem_zero, sem_io, sem_w,
):
    mark = _Marks()
    row8 = lax.broadcasted_iota(jnp.int32, (8, T), 0)
    unit_of_row = row8 & 3
    second = row8 >= 4

    def rows(j):
        return pl.ds(pl.multiple_of(j * T, T), T)

    class Step:
        def __init__(self, src, dst):
            self.src, self.dst = src, dst
            self.n = 4

        def start(self, sem):
            if DEBUG.get("no_read_dma"):
                return
            n = self.n
            pltpu.make_async_copy(self.src(0, n - 1), self.dst(0, n - 1), sem).start(priority=1)
            pltpu.make_async_copy(self.src(n - 1, 1), self.dst(n - 1, 1), sem).start(priority=0)

        def wait(self, sem):
            if DEBUG.get("no_read_dma"):
                return
            pltpu.make_async_copy(self.src(0, self.n), self.dst(0, self.n), sem).wait()

    def step_a(src, head, dst, unit0, j):
        return Step(lambda r, n: src.at[pl.ds(4 * head + r, n), rows(j)],
                    lambda r, n: dst.at[pl.ds(unit0 + r, n), rows(j)])

    def step_b(src, group, dst, unit0, j):
        return Step(lambda r, n: src.at[pl.ds(4 * group + r, n), 3, rows(j)],
                    lambda r, n: dst.at[pl.ds(unit0 + r, n), rows(j)])

    def wq_piece(ref, t):
        rr = pl.ds(pl.multiple_of((t >> 2) * 16, 16), 16)
        cc = pl.ds(pl.multiple_of((t & 3) * 1024, 1024), 1024)
        return lambda r, n: ref.at[pl.ds(r, n), rr, cc]

    def wo_piece(ref, t):
        rr = pl.ds(pl.multiple_of(t * 32, 32), 32)
        return lambda r, n: ref.at[pl.ds(r, n), rr]

    def step_wq(src, dst, t):
        st = Step(wq_piece(src, t), wq_piece(dst, t))
        st.n = 5
        return st

    def step_wo(src, dst, t):
        return Step(wo_piece(src, t), wo_piece(dst, t))

    def zero_copy(dst, i, sem):
        ngrp = H // ZSEG
        grp = i & (ngrp - 1)
        rest = i >> (ngrp.bit_length() - 1)
        j = rest & (NT - 1)
        quarter = rest >> 4
        return pltpu.make_async_copy(
            zeros, dst.at[pl.ds(grp * ZSEG, ZSEG), quarter, rows(j)], sem)

    def zero_fill(lo, hi, sem, wait=False):
        assert lo % 2 == 0 and hi % 2 == 0

        def body(i, _):
            for dst in (dkb_hbm, dvb_hbm):
                cp = zero_copy(dst, i, sem)
                cp.wait() if wait else cp.start()

        lax.fori_loop(lo // 2, hi // 2, body, None)

    def blocks_f32(v8):
        return jnp.concatenate(
            [jnp.where(unit_of_row == r, v8, 0.0) for r in range(4)], axis=1)

    def blocks(v8):
        return blocks_f32(v8).astype(BF16)

    def dot_keys(lhs, ref, unit0, j):
        x = jnp.concatenate([ref[unit0 + r, rows(j), :] for r in range(4)], axis=1)
        return lax.dot_general(lhs, x, _NT_DIMS, preferred_element_type=F32)

    def tiles(ref, unit0, j):
        return ref[pl.ds(unit0, 4), rows(j), :].reshape(4 * T, DH)

    def over_units(x, per_head, op):
        red = jnp.max if op == "max" else jnp.sum
        x = red(x, axis=1, keepdims=True)
        if per_head:
            return x
        fill = -jnp.inf if op == "max" else 0.0
        sec = lax.broadcasted_iota(jnp.int32, (8, 1), 0) >= 4
        lo = red(jnp.where(sec, fill, x), axis=0, keepdims=True)
        hi = red(jnp.where(sec, x, fill), axis=0, keepdims=True)
        return jnp.where(sec, hi, lo)

    def tree(op, xs):
        while len(xs) > 1:
            xs = [op(xs[i], xs[i + 1]) for i in range(0, len(xs), 2)]
        return xs[0]

    def softmax(per_head):
        s = [s_buf[j] * SCALE for j in range(NT)]
        m = over_units(tree(jnp.maximum, s), per_head, "max")
        e = [jnp.exp(x - m) for x in s]
        inv = 1.0 / over_units(tree(jnp.add, e), per_head, "sum")
        for j in range(NT):
            p_cur[j] = e[j] * inv

    def pair_a(first_ref, second_ref, head):
        a = jnp.broadcast_to(first_ref[pl.ds(head, 1), :], (8, DH))
        b = jnp.broadcast_to(second_ref[pl.ds(head, 1), :], (8, DH))
        return jnp.where(second, b, a)

    def m_init():
        return jnp.zeros((DH + 16, DH), F32), jnp.zeros((8, DH), F32)

    def m_step(k_unit, v_unit, j, carry, loaded=None):
        acc, oacc = carry
        pk = blocks_f32(p_cur[j])
        v4 = tiles(va, v_unit, j)
        k4 = tiles(pool, k_unit, j)
        p_row = jnp.concatenate([p_cur[j, pl.ds(4 + r, 1), :] for r in range(4)], axis=1)
        if loaded is not None:
            loaded()
        lhs = jnp.concatenate([v4.T.astype(F32) * p_row, pk, jnp.zeros_like(pk)], axis=0)
        acc = acc + jnp.dot(lhs.astype(BF16), k4, preferred_element_type=F32)
        oacc = oacc + jnp.dot(pk.astype(BF16), v4, preferred_element_type=F32)
        return acc, oacc

    def m_finish(carry):
        acc, oacc = carry
        o = jnp.sum(jnp.where(second, oacc, 0.0), axis=0, keepdims=True)
        kbar = jnp.sum(jnp.where(second, acc[DH:DH + 8], 0.0), axis=0, keepdims=True)
        o_col = jnp.broadcast_to(o, (DH, DH)).T
        return o, (acc[:DH] - o_col * kbar).astype(BF16)

    def cols(c):
        return pl.ds(pl.multiple_of(c * 1024, 1024), 1024)

    def rows8(v):
        return jnp.broadcast_to(v, (8, v.shape[1])).astype(BF16)

    def store_a(dst):
        def store(c, res):
            v = res[:, :DH]
            for i in range(1, 8):
                v = jnp.where(row8 == i, res[:, i * DH:(i + 1) * DH], v)
            dst[pl.ds(pl.multiple_of(c * 8, 8), 8), :] = v
        return store

    def store_b(dst, keep):
        def store(c, res):
            for k in range(2):
                v = res[:, 4 * k * DH:(4 * k + 1) * DH]
                for r in range(1, 4):
                    v = jnp.where(unit_of_row == r,
                                  res[:, (4 * k + r) * DH:(4 * k + r + 1) * DH], v)
                if keep is not None:
                    v = jnp.where(keep, dst[2 * c + k], v)
                dst[2 * c + k] = v
        return store

    def spread_a(src):
        def spread(c):
            v = src[pl.ds(pl.multiple_of(c * 8, 8), 8), :]
            return jnp.concatenate([jnp.where(row8 == i, v, 0.0) for i in range(8)], axis=1)
        return spread

    def spread_b(src, select):
        def spread(c):
            out = []
            for k in range(2):
                v = src[2 * c + k]
                if select is not None:
                    v = jnp.where(select, v, 0.0)
                out.append(blocks_f32(v))
            return jnp.concatenate(out, axis=1)
        return spread

    def to_heads_wq(v, wq, store):
        lhs = rows8(v)

        def body(c, _):
            w = wq[:, :, cols(c)].reshape(D, 1024)
            store(c, jnp.dot(lhs, w, preferred_element_type=F32))
        lax.fori_loop(0, 4, body, None)

    def to_heads_wo(v, wo, store):
        lhs = rows8(v)

        def body(c, _):
            store(c, lax.dot_general(lhs, wo[c], _NT_DIMS, preferred_element_type=F32))
        lax.fori_loop(0, 4, body, None)

    def from_heads_wo(spread, wo):
        def body(c, acc):
            return acc + jnp.dot(spread(c).astype(BF16), wo[c], preferred_element_type=F32)
        acc = lax.fori_loop(0, 4, body, jnp.zeros((8, D), F32))
        return jnp.sum(acc, axis=0, keepdims=True)

    def from_heads_wq(spread, wq):
        def body(c, acc):
            w = wq[:, :, cols(c)].reshape(D, 1024)
            return acc + lax.dot_general(spread(c).astype(BF16), w, _NT_DIMS,
                                         preferred_element_type=F32)
        acc = lax.fori_loop(0, 4, body, jnp.zeros((8, D), F32))
        return jnp.sum(acc, axis=0, keepdims=True)

    def layernorm(x, i):
        xc = x - jnp.mean(x, axis=1, keepdims=True)
        inv = 1.0 / jnp.sqrt(jnp.mean(xc * xc, axis=1, keepdims=True) + EPS)
        y = xc * inv
        vec[pl.ds(V_H + i, 1), :] = y
        vec[pl.ds(V_INV + i, 1), :] = jnp.broadcast_to(inv, (1, D))
        return y

    def layernorm_bwd(dy, i):
        y = vec[pl.ds(V_H + i, 1), :]
        inv = vec[pl.ds(V_INV + i, 1), :]
        return inv * (dy - jnp.mean(dy, axis=1, keepdims=True)
                      - y * jnp.mean(dy * y, axis=1, keepdims=True))

    def stage(a_now, a_next, work_a, b_now, b_next, work_b, carry=None, span=None):
        def light(j, carry):
            a_now(j).wait(sem_a.at[j])
            if a_next is not None:
                a_next(j).start(sem_a.at[j])
            if work_a is not None:
                s_buf[j] = work_a(j)
            b_now(j).wait(sem_b.at[j])
            if b_next is not None:
                b_next(j).start(sem_b.at[j])
            if work_b is not None:
                carry = work_b(j, carry)
            return carry

        def heavy(i, carry):
            js = [span * i + k for k in range(span)]
            for j in js:
                a_now(j).wait(sem_a.at[j])
                b_now(j).wait(sem_b.at[j])
            pending = []
            for j in js:
                a_next(j).start(sem_a.at[j])
                if work_a is not None:
                    pending.append((j, work_a(j)))
                carry = work_b(j, carry, lambda: b_next(j).start(sem_b.at[j]))
            for j, value in pending:
                s_buf[j] = value
            return carry

        if span is None:
            return lax.fori_loop(0, NT, light, carry)
        return lax.fori_loop(0, NT // span, heavy, carry)

    def scores(lhs, unit0):
        return lambda j: dot_keys(lhs, pool, unit0, j)

    def all_scores(lhs, unit0):
        def body(j, _):
            s_buf[j] = dot_keys(lhs, pool, unit0, j)
        lax.fori_loop(0, NT, body, None, unroll=4)

    wqa_a = lambda j: step_wq(wqa_hbm, wqa, 2 * j)
    wqa_b = lambda j: step_wq(wqa_hbm, wqa, 2 * j + 1)
    x_cp = pltpu.make_async_copy(x_hbm, x_in, sem_io.at[0])
    g_cp = pltpu.make_async_copy(g_hbm, g_in, sem_io.at[1])

    def first(j, _):
        wqa_a(j).start(sem_a.at[j])
        wqa_b(j).start(sem_b.at[j])
    mark("start")
    lax.fori_loop(0, NT, first, None)
    x_cp.start()
    g_cp.start()
    for i, s in enumerate(A_SLOT):
        tab[TAB_A + i] = 4 * s
    for i, s in enumerate(KB_SLOT):
        tab[TAB_KB + i] = 4 * s
    for i, s in enumerate(STAGE_SLOT[:2 * NSTAGE]):
        tab[TAB_STAGE + i] = 4 * s
    zeros[...] = jnp.zeros(zeros.shape, BF16)

    def head1(n):
        return (n + NRES) & (H - 1)

    slot0 = (NRES - H) % NSLOT

    def next_slot(s):
        return jnp.where(s == NSLOT - 1, 0, s + 1)

    def ka_steps(n, s):
        return lambda j: step_a(ka_hbm, head1(n), pool, 4 * s, j)

    def va_steps(n):
        return lambda j: step_a(va_hbm, head1(n), va, 4 * head1(n), j)

    woa_lo = lambda j: step_wo(woa_hbm, woa, j)
    woa_hi = lambda j: step_wo(woa_hbm, woa, NT + j)
    wqb_a = lambda j: step_wq(wqb_hbm, wqb, 2 * j)
    wqb_b = lambda j: step_wq(wqb_hbm, wqb, 2 * j + 1)
    wob_lo = lambda j: step_wo(wob_hbm, wob, j)
    wob_hi = lambda j: step_wo(wob_hbm, wob, NT + j)

    stage(wqa_a, ka_steps(0, slot0), None, wqa_b, woa_lo, None)
    mark("q1")
    x_cp.wait()
    g_cp.wait()
    x0 = x_in[0].astype(F32)
    g4 = g_in[0].astype(F32)
    vec[pl.ds(V_G + 3, 1), :] = g4
    to_heads_wq(layernorm(x0, 0), wqa, store_a(qa1))

    def q1_lhs(n):
        return blocks(pair_a(qa1, qa1, head1(n)))

    mark("k0")
    stage(ka_steps(0, slot0), ka_steps(1, (slot0 + 1) % NSLOT), scores(q1_lhs(0), 4 * slot0),
          woa_lo, va_steps(0), None)
    softmax(False)

    def finish1(n, carry):
        o, m = m_finish(carry)
        oa1[pl.ds(head1(n), 1), :] = o
        m1[head1(n)] = m

    def head_first_use(n, s, a_next, b_next):
        s1 = next_slot(s)
        carry = stage(
            ka_steps(n + 1, s1), a_next(next_slot(s1)), scores(q1_lhs(n + 1), 4 * s1),
            va_steps(n), b_next,
            lambda j, c, f: m_step(4 * s, 4 * head1(n), j, c, f), m_init(), SPAN)
        finish1(n, carry)
        softmax(False)
        return s1

    mark("a1")
    lax.fori_loop(
        0, H - 2,
        lambda n, s: head_first_use(n, s, lambda s2: ka_steps(n + 2, s2), va_steps(n + 1)),
        jnp.int32(slot0))
    mark("a1_30")
    head_first_use(H - 2, jnp.int32((slot0 + H - 2) % NSLOT), lambda s2: woa_hi, va_steps(H - 1))
    mark("a1_31")
    carry = stage(
        woa_hi, wqb_a, None, va_steps(H - 1), wqb_b,
        lambda j, c, f: m_step(4 * ((slot0 + H - 1) % NSLOT), 4 * head1(H - 1), j, c, f),
        m_init(), SPAN)
    mark("x1")
    finish1(H - 1, carry)
    x1 = x0 + from_heads_wo(spread_a(oa1), woa)

    def kb_unit1(g):
        return 4 * (NRES + (g & 1))

    def kb_steps(g):
        return lambda j: step_b(kb_hbm, g, pool, kb_unit1(g), j)

    def vb_steps(g):
        return lambda j: step_b(vb_hbm, g, vb, 4 * g, j)

    mark("b1")
    h2 = layernorm(x1, 1)
    stage(wqb_a, kb_steps(0), None, wqb_b, wob_lo, None)
    mark("q2")
    to_heads_wq(h2, wqb, store_b(qb, None))
    mark("kb0")
    stage(kb_steps(0), kb_steps(1), scores(blocks(qb[0]), kb_unit1(0)),
          wob_lo, vb_steps(0), None)
    softmax(True)

    def pv(g):
        def work(j, acc):
            return acc + jnp.dot(blocks(p_cur[j]), tiles(vb, 4 * g, j),
                                 preferred_element_type=F32)
        return work

    def group_first_use(g, a_next):
        ob[g] = stage(kb_steps(g + 1), a_next, scores(blocks(qb[g + 1]), kb_unit1(g + 1)),
                      vb_steps(g), vb_steps(g + 1), pv(g), jnp.zeros((8, DH), F32))
        softmax(True)

    mark("b1_main")
    lax.fori_loop(0, NG - 2, lambda g, _: group_first_use(g, kb_steps(g + 2)), None)
    mark("b1_tail")
    group_first_use(NG - 2, wob_hi)
    ob[NG - 1] = stage(wob_hi, None, None, vb_steps(NG - 1), None, pv(NG - 1),
                       jnp.zeros((8, DH), F32))
    mark("x2")
    zero_fill(0, NZERO_EARLY, sem_zero.at[0])
    x2 = x1 + from_heads_wo(spread_b(ob, ~second), wob)

    to_heads_wq(layernorm(x2, 2), wqa, store_a(qa3))

    def pm_place(head):
        unit = jnp.where(head < 16, 4 * PM_SLOT[0], 4 * PM_SLOT[1]) + ((head & 15) >> 2)
        return unit, (head & 3) * 512

    def p_rows(row0, j):
        return pl.ds(pl.multiple_of(row0 + 16 * j, 16), 16)

    def keep_p(unit, row0):
        for j in range(NT):
            pool[unit, p_rows(row0, j), :] = pltpu.bitcast(p_cur[j], BF16)

    def slot_ref(unit0):
        return pool.at[pl.ds(unit0, 4)]

    def reread_a(head):
        unit0 = tab[TAB_A + head]
        return pltpu.make_async_copy(
            ka_hbm.at[pl.ds(4 * head, 4)], slot_ref(unit0), sem_slot.at[unit0 >> 2])

    def reread_b(g):
        unit0 = tab[TAB_KB + g]
        return pltpu.make_async_copy(
            kb_hbm.at[pl.ds(4 * g, 4), 3], slot_ref(unit0), sem_slot.at[unit0 >> 2])

    def refill(h):
        if REFILL[h]:
            kind, idx = REFILL[h]
            (reread_a if kind == "A" else reread_b)(idx).start()

    def q3_lhs(head):
        return blocks(pair_a(qa1, qa3, head))

    def finish3(head, carry):
        o, m = m_finish(carry)
        oa3[pl.ds(head, 1), :] = o
        unit, row0 = pm_place(head)
        keep_p(unit, row0)
        pool[unit, pl.ds(pl.multiple_of(row0 + 256, DH), DH), :] = m

    def head_second_use(head, wait_next):
        if wait_next:
            reread_a(head + 1).wait()
        lhs = q3_lhs(head + 1)
        k_next, k_now = tab[TAB_A + head + 1], tab[TAB_A + head]

        def body(j, carry):
            s_buf[j] = dot_keys(lhs, pool, k_next, j)
            return m_step(k_now, 4 * head, j, carry)
        finish3(head, lax.fori_loop(0, NT, body, m_init(), unroll=UNROLL3))
        softmax(False)

    all_scores(q3_lhs(0), 4 * A_SLOT[0])
    softmax(False)
    mark("a3_early")
    lax.fori_loop(0, READS_AFTER_HEAD + 1, lambda h, _: head_second_use(h, False), None)
    mark("zwait")
    zero_fill(0, NZERO_EARLY, sem_zero.at[0], wait=True)
    for h in range(READS_AFTER_HEAD + 1):
        refill(h)

    def head_and_refill(h, _):
        @pl.when(h + 1 >= NRES)
        def _():
            reread_a(h + 1).wait()
        head_second_use(h, False)
        skipped = 1 + (h >> 4)

        @pl.when((h & 15) != 0)
        def _():
            @pl.when(h < FIRST_B_REFILL)
            def _():
                reread_a(NRES + h - skipped).start()

            @pl.when(h >= FIRST_B_REFILL)
            def _():
                reread_b(h - FIRST_B_REFILL).start()

    mark("a3_main")
    lax.fori_loop(READS_AFTER_HEAD + 1, LAST_REFILL + 1, head_and_refill, None)
    mark("rwait")
    for h in range(LAST_REFILL + 2, H):
        reread_a(h).wait()
    for g in range(NG - 2):
        reread_b(g).wait()
    mark("a3_late")
    z1 = NZERO_EARLY + 60
    z2 = z1 + 50
    zero_fill(NZERO_EARLY, z1, sem_zero.at[1])
    lax.fori_loop(LAST_REFILL + 1, H - 1, lambda h, _: head_second_use(h, False), None)
    finish3(H - 1, lax.fori_loop(
        0, NT, lambda j, c: m_step(4 * A_SLOT[H - 1], 4 * (H - 1), j, c), m_init()))
    x3 = x2 + from_heads_wo(spread_a(oa3), woa)

    mark("b4")
    to_heads_wq(layernorm(x3, 3), wqb, store_b(qb, second == False))
    to_heads_wo(g4, wob, store_b(dob, None))

    def pb_place(g):
        return 4 * PB_SLOT, g * 256

    def load_p(unit, row0, j):
        return pltpu.bitcast(pool[unit, p_rows(row0, j), :], F32)

    def dprobs(do_lhs, v_ref, v_unit, p_unit, p_row0, per_head):
        def body(j, dsum):
            dp = dot_keys(do_lhs, v_ref, v_unit, j)
            s_buf[j] = dp
            return dsum + load_p(p_unit, p_row0, j) * dp
        dsum = lax.fori_loop(0, NT, body, jnp.zeros((8, T), F32), unroll=4)
        return over_units(dsum, per_head, "sum")

    def dq_group(g):
        unit, row0 = pb_place(g)
        delta = dprobs(blocks(dob[g]), vb, 4 * g, unit, row0, True)
        k_unit = tab[TAB_KB + g]

        def body(j, acc):
            ds = load_p(unit, row0, j) * (s_buf[j] - delta) * SCALE
            return acc + jnp.dot(blocks(ds), tiles(pool, k_unit, j), preferred_element_type=F32)
        dqb[g] = lax.fori_loop(0, NT, body, jnp.zeros((8, DH), F32), unroll=4)

    def group_second_use(g, _):
        all_scores(blocks(qb[g]), tab[TAB_KB + g])
        softmax(True)
        keep_p(*pb_place(g))
        ob[g] = lax.fori_loop(0, NT, pv(g), jnp.zeros((8, DH), F32), unroll=4)
        dq_group(g)

    lax.fori_loop(0, NG, group_second_use, None)
    mark("z1")
    zero_fill(z1, z2, sem_zero.at[1])
    x4 = x3 + from_heads_wo(spread_b(ob, second), wob)
    out_st[0] = x4.astype(BF16)
    out_cp = pltpu.make_async_copy(out_st, out_hbm, sem_io.at[0])
    out_cp.start()

    def dq_heads(do_ref, dq_ref, matrix):
        def body(c, _):
            m = jnp.concatenate([matrix(8 * c + i) for i in range(8)], axis=0)
            dq = jnp.dot(spread_a(do_ref)(c).astype(BF16), m, preferred_element_type=F32)
            dq_ref[pl.ds(pl.multiple_of(c * 8, 8), 8), :] = dq * SCALE
        lax.fori_loop(0, 4, body, None)

    def m3(head):
        unit, row0 = pm_place(head)
        return pool[unit, pl.ds(pl.multiple_of(row0 + 256, DH), DH), :]

    mark("bwd")
    g3 = g4 + layernorm_bwd(from_heads_wq(spread_b(dqb, second), wqb), 3)
    vec[pl.ds(V_G + 2, 1), :] = g3
    to_heads_wo(g3, woa, store_a(doa3))
    dq_heads(doa3, dqa3, m3)
    g2 = g3 + layernorm_bwd(from_heads_wq(spread_a(dqa3), wqa), 2)
    vec[pl.ds(V_G + 1, 1), :] = g2
    to_heads_wo(g2, wob, store_b(dob, second))
    lax.fori_loop(0, NG, lambda g, _: dq_group(g), None)
    mark("z2")
    zero_fill(z2, NZERO, sem_zero.at[1])
    mark("bwd1")
    g1 = g2 + layernorm_bwd(from_heads_wq(spread_b(dqb, ~second), wqb), 1)
    vec[pl.ds(V_G + 0, 1), :] = g1
    to_heads_wo(g1, woa, store_a(doa1))
    dq_heads(doa1, dqa1, lambda head: m1[head])
    g0 = g1 + layernorm_bwd(from_heads_wq(spread_a(dqa1), wqa), 0)
    dx_st[0] = g0.astype(BF16)
    dx_cp = pltpu.make_async_copy(dx_st, dx_hbm, sem_io.at[1])
    dx_cp.start()

    def vec_rows(i, n):
        return jnp.broadcast_to(vec[pl.ds(i, 1), :], (n, D))

    def weight_grads(wq, wo, h_rows, g_rows, dq_spread, o_spread):
        h_lhs, g_rhs = h_rows.astype(BF16), g_rows.astype(BF16)

        def body(c, _):
            dq, o = dq_spread(c), o_spread(c)
            for i in range(8):
                head = slice(i * DH, (i + 1) * DH)
                dq_i = dq[:, head].astype(BF16)
                head_cols = pl.ds(pl.multiple_of(c * 1024 + i * DH, DH), DH)
                for b in range(D // 128):
                    wq[b, :, head_cols] = lax.dot_general(
                        h_lhs[:, b * 128:(b + 1) * 128], dq_i, _TN_DIMS,
                        preferred_element_type=F32).astype(BF16)
                wo[c, head, :] = lax.dot_general(
                    o[:, head].astype(BF16), g_rhs, _TN_DIMS,
                    preferred_element_type=F32).astype(BF16)
        lax.fori_loop(0, 4, body, None)

    def both(first_ref, second_ref):
        return lambda c: jnp.concatenate(
            [spread_a(first_ref)(c), spread_a(second_ref)(c)], axis=0)

    def pair_b(i, k):
        sec = lax.broadcasted_iota(jnp.int32, (8, D), 0) >= 4
        return jnp.where(sec, vec_rows(k, 8), vec_rows(i, 8))

    mark("dw")
    weight_grads(wqa, woa,
                 jnp.concatenate([vec_rows(V_H + 0, 8), vec_rows(V_H + 2, 8)], axis=0),
                 jnp.concatenate([vec_rows(V_G + 0, 8), vec_rows(V_G + 2, 8)], axis=0),
                 both(dqa1, dqa3), both(oa1, oa3))
    weight_grads(wqb, wob, pair_b(V_H + 1, V_H + 3), pair_b(V_G + 1, V_G + 3),
                 spread_b(dqb, None), spread_b(ob, None))

    weights_out = ((wqa, dwqa_hbm, wq_piece, 5), (woa, dwoa_hbm, wo_piece, 4),
                   (wqb, dwqb_hbm, wq_piece, 5), (wob, dwob_hbm, wo_piece, 4))

    def write_weights(t, _):
        for i, (src, dst, piece, n) in enumerate(weights_out):
            pltpu.make_async_copy(piece(src, t)(0, n), piece(dst, t)(0, n), sem_w.at[i]).start()
    mark("dw_issue")
    lax.fori_loop(0, 2 * NT, write_weights, None)

    def stage_wait(unit0):
        pltpu.make_async_copy(slot_ref(unit0), slot_ref(unit0), sem_slot.at[unit0 >> 2]).wait()

    def outer_products(coef, vectors, unit0):
        lhs = jnp.concatenate(coef, axis=0).T.astype(BF16)
        zero = jnp.zeros_like(vectors)
        halves = (jnp.concatenate([vectors, zero], axis=0).astype(BF16),
                  jnp.concatenate([zero, vectors], axis=0).astype(BF16))
        zero16 = jnp.zeros((16, 4 * DH), BF16)
        for j in range(NT):
            rhs = jnp.concatenate(
                [halves[j % 2] if k == j // 2 else zero16 for k in range(NT // 2)], axis=0)
            res = jnp.dot(lhs, rhs, preferred_element_type=F32)
            for r in range(4):
                pool[unit0 + r, pl.ds(j * T, T), :] = res[:, r * DH:(r + 1) * DH].astype(BF16)

    def kv_grads(n, k, do8, q8, v_ref, v_unit, p_place, per_head, dk_dst, dv_dst):
        unit, row0 = p_place
        delta = dprobs(blocks(do8), v_ref, v_unit, unit, row0, per_head)
        sk, sv = tab[TAB_STAGE + 2 * k], tab[TAB_STAGE + 2 * k + 1]

        if not DEBUG.get("no_kv_dma"):
            @pl.when(n >= NSTAGE)
            def _():
                stage_wait(sk)
                stage_wait(sv)

        p = [load_p(unit, row0, j) for j in range(NT)]
        ds = [p[j] * (s_buf[j] - delta) * SCALE for j in range(NT)]
        if not DEBUG.get("no_kv_compute"):
            outer_products(ds, blocks_f32(q8), sk)
            outer_products(p, blocks_f32(do8), sv)

        def issue(j, _):
            for st, dst in ((sk, dk_dst), (sv, dv_dst)):
                pltpu.make_async_copy(pool.at[pl.ds(st, 4), rows(j)], dst(j),
                                      sem_slot.at[st >> 2]).start()
        if not DEBUG.get("no_kv_dma"):
            lax.fori_loop(0, NT, issue, None, unroll=2)
        return jnp.where(k == NSTAGE - 1, 0, k + 1)

    def grads_b(g, k):
        return kv_grads(g, k, dob[g], qb[g], vb, 4 * g, pb_place(g), True,
                        lambda j: dkb_hbm.at[pl.ds(4 * g, 4), 3, rows(j)],
                        lambda j: dvb_hbm.at[pl.ds(4 * g, 4), 3, rows(j)])

    def grads_a(h, k):
        return kv_grads(NG + h, k, pair_a(doa1, doa3, h), pair_a(qa1, qa3, h), va, 4 * h,
                        pm_place(h), False,
                        lambda j: dka_hbm.at[pl.ds(4 * h, 4), rows(j)],
                        lambda j: dva_hbm.at[pl.ds(4 * h, 4), rows(j)])

    mark("kv_b")
    k = lax.fori_loop(0, NG, grads_b, jnp.int32(0))
    mark("kv_a")
    lax.fori_loop(0, H, grads_a, k)

    mark("drain")
    out_cp.wait()
    dx_cp.wait()
    zero_fill(NZERO_EARLY, NZERO, sem_zero.at[1], wait=True)
    for i, (src, dst, _, _) in enumerate(weights_out):
        pltpu.make_async_copy(src, dst, sem_w.at[i]).wait()
    for s in STAGE_SLOT[:2 * NSTAGE]:
        if DEBUG.get("no_kv_dma"):
            cp = pltpu.make_async_copy(pool.at[pl.ds(4 * s, 4), rows(0)], dka_hbm.at[pl.ds(4 * s, 4), rows(0)], sem_slot.at[s])
            cp.start()
            cp.wait()
        else:
            stage_wait(4 * s)
    mark(None)


@jax.jit
def pallas_interleave_layers__gqa_block_cached__sliding_block_cached__decode_kernel(
    A_x: jax.Array,
    A_k_cache: jax.Array,
    A_v_cache: jax.Array,
    A_wq: jax.Array,
    A_wo: jax.Array,
    B_x: jax.Array,
    B_k_cache: jax.Array,
    B_v_cache: jax.Array,
    B_wq: jax.Array,
    B_wo: jax.Array,
    grad_out: jax.Array,
):
    del B_x
    cache_shape = A_k_cache.shape
    a_view = (4 * H, UNIT, DH)
    b_view = (H, 4, UNIT, DH)
    wq_view = (5, 128, H * DH)
    wo_view = (4, 1024, D)

    def sds(shape):
        return jax.ShapeDtypeStruct(shape, BF16)

    heads_a = pltpu.VMEM((H, DH), F32)
    heads_b = pltpu.VMEM((NG, 8, DH), F32)
    io = pltpu.VMEM((1, 1, D), BF16)
    hbm = pl.BlockSpec(memory_space=pl.ANY)
    outs = pl.pallas_call(
        _kernel,
        out_shape=[sds((1, 1, D)), sds((1, 1, D)),
                   sds(a_view), sds(a_view), sds(wq_view), sds(wo_view),
                   sds(b_view), sds(b_view), sds(wq_view), sds(wo_view)],
        in_specs=[hbm] * 10,
        out_specs=[hbm] * 10,
        scratch_shapes=[
            pltpu.VMEM(a_view, BF16),
            pltpu.VMEM((H, UNIT, DH), BF16),
            pltpu.VMEM(wq_view, BF16), pltpu.VMEM(wo_view, BF16),
            pltpu.VMEM(wq_view, BF16), pltpu.VMEM(wo_view, BF16),
            pltpu.VMEM((4 * NSLOT, UNIT, DH), BF16),
            pltpu.VMEM((H, DH, DH), BF16),
            pltpu.VMEM((ZSEG, T, DH), BF16),
            pltpu.VMEM((NT, 8, T), F32),
            pltpu.VMEM((NT, 8, T), F32),
            *[heads_a] * 8, *[heads_b] * 4,
            pltpu.VMEM((16, D), F32),
            io, io, io, io,
            pltpu.SMEM((TAB_SIZE,), jnp.int32),
            pltpu.SemaphoreType.DMA((NT,)), pltpu.SemaphoreType.DMA((NT,)),
            pltpu.SemaphoreType.DMA((NSLOT,)), pltpu.SemaphoreType.DMA((2,)),
            pltpu.SemaphoreType.DMA((2,)), pltpu.SemaphoreType.DMA((4,)),
        ],
        compiler_params=pltpu.CompilerParams(vmem_limit_bytes=128 * 1024 * 1024),
    )(A_x, grad_out,
      A_k_cache.reshape(a_view), A_v_cache.reshape(a_view),
      A_wq.reshape(wq_view), A_wo.reshape(wo_view),
      B_k_cache.reshape(b_view), B_v_cache.reshape(b_view),
      B_wq.reshape(wq_view), B_wo.reshape(wo_view))
    out, dx, dka, dva, dwqa, dwoa, dkb, dvb, dwqb, dwob = outs
    return (out, dx,
            dka.reshape(cache_shape), dva.reshape(cache_shape),
            dwqa.reshape(A_wq.shape), dwoa.reshape(A_wo.shape),
            dkb.reshape(cache_shape), dvb.reshape(cache_shape),
            dwqb.reshape(B_wq.shape), dwob.reshape(B_wo.shape))
```

```python
import jax
import jax.numpy as jnp
from jax import lax
import jax.experimental.pallas as pl
import jax.experimental.pallas.tpu as pltpu

F32 = jnp.float32
BF16 = jnp.bfloat16

D = 640
H = 32
DH = 128
T = 128
NT = 16
NG = H // 4
SCALE = DH ** -0.5
EPS = 1e-5

NSLOT = 13
NRES = NSLOT - 2
VB0 = 4 * H

_NT_DIMS = (((1,), (1,)), ((), ()))
_TN_DIMS = (((0,), (0,)), ((), ()))


def _slot_plan():
    slot = list(range(NRES))
    kb_slot = [None] * NG
    kb_slot[NG - 2], kb_slot[NG - 1] = NRES, NRES + 1
    pm_slot = []
    refill = []
    todo = [("A", h) for h in range(NRES, H)] + [("B", g) for g in range(NG - 2)]
    for h in range(H):
        if h % 16 == 0:
            pm_slot.append(slot[h])
            refill.append(None)
        elif todo:
            kind, idx = todo.pop(0)
            refill.append((kind, idx))
            if kind == "A":
                slot.append(slot[h])
            else:
                kb_slot[idx] = slot[h]
        else:
            refill.append(None)
    assert not todo and len(slot) == H
    stage = [s for s in range(NSLOT) if s not in pm_slot]
    return slot, kb_slot, pm_slot, refill, stage


A_SLOT, KB_SLOT, PM_SLOT, REFILL, STAGE_SLOT = _slot_plan()
NSTAGE = len(STAGE_SLOT) // 2
ZERO_UNIT = 4 * PM_SLOT[0] + 3
PB_UNIT = 4 * PM_SLOT[1] + 3

NZERO = 3 * 4 * NT
LEAD_E2, LEAD_E3, LEAD_E4 = 1, 1, 4
NZERO_FIRST = 12
NZERO_EARLY = 20
FIRST_READER = 4
CATCH_UP = 1
IN_FLIGHT = 2

TAB_A = 0
TAB_KB = TAB_A + H
TAB_READ = TAB_A + NRES
TAB_STAGE = TAB_KB + NG
TAB_SIZE = TAB_STAGE + 2 * NSTAGE

V_H, V_G = 0, 4


def _kernel(
    x_hbm, g_hbm, ka_hbm, va_hbm, wqa_hbm, woa_hbm, kb_hbm, vb_hbm, wqb_hbm, wob_hbm,
    out_hbm, dx_hbm, dka_hbm, dva_hbm, dwqa_hbm, dwoa_hbm, dkb_hbm, dvb_hbm, dwqb_hbm, dwob_hbm,
    vbuf, wqa, woa, wqb, wob, pool, m1, zeros, s_buf, p_cur,
    qa, oa, doa, dqa, qb, ob, dob, dqb, vec, inv_std,
    x_io, g_io, tab,
    sem_a, sem_b, sem_slot, sem_zero, sem_io, sem_w,
):
    row8 = lax.broadcasted_iota(jnp.int32, (8, T), 0)
    unit_of_row = row8 & 3
    second = row8 >= 4

    class Step:
        def __init__(self, src, dst, n=4):
            self.src, self.dst, self.n = src, dst, n

        def start(self, sem):
            n = self.n
            pltpu.make_async_copy(self.src(0, n - 1), self.dst(0, n - 1), sem).start(priority=1)
            pltpu.make_async_copy(self.src(n - 1, 1), self.dst(n - 1, 1), sem).start(priority=0)

        def wait(self, sem):
            pltpu.make_async_copy(self.src(0, self.n), self.dst(0, self.n), sem).wait()

    def step_a(src, head, dst, unit0, j):
        return Step(lambda r, n: src.at[pl.ds(4 * head + r, n), j],
                    lambda r, n: dst.at[pl.ds(unit0 + r, n), j])

    def step_b(src, group, dst, unit0, j):
        return Step(lambda r, n: src.at[group, pl.ds(r, n), 3, j],
                    lambda r, n: dst.at[pl.ds(unit0 + r, n), j])

    def wq_piece(ref, t):
        rr = pl.ds(pl.multiple_of((t >> 1) * 8, 8), 8)
        cc = pl.ds(pl.multiple_of((t & 1) * 2048, 2048), 2048)
        return lambda r, n: ref.at[pl.ds(r, n), rr, cc]

    def wo_piece(ref, t):
        rr = pl.ds(pl.multiple_of(t * 32, 32), 32)
        return lambda r, n: ref.at[pl.ds(r, n), rr]

    def step_wq(src, dst, t):
        return Step(wq_piece(src, t), wq_piece(dst, t), 5)

    def step_wo(src, dst, t):
        return Step(wo_piece(src, t), wo_piece(dst, t))

    def zero_fill(lo, hi, sem, early=False, wait=False):
        def body(i, _):
            j, head, quarter = i & (NT - 1), (i >> 4) & 3, i >> 6
            for dst in (dkb_hbm, dvb_hbm):
                if early:
                    copies = [(zeros, dst.at[pl.ds(4 * k, 4), head, quarter, j]) for k in range(2)]
                else:
                    copies = [(pool.at[ZERO_UNIT, pl.ds(0, NG)], dst.at[:, head, quarter, j])]
                for src, dst_block in copies:
                    cp = pltpu.make_async_copy(src, dst_block, sem)
                    cp.wait() if wait else cp.start()

        lax.fori_loop(lo, hi, body, None)

    def blocks_f32(v8):
        return jnp.concatenate(
            [jnp.where(unit_of_row == r, v8, 0.0) for r in range(4)], axis=1)

    def blocks(v8):
        return blocks_f32(v8).astype(BF16)

    def dot_keys(lhs, ref, unit0, j, stride=1):
        x = jnp.concatenate([ref[unit0 + r * stride, j] for r in range(4)], axis=1)
        return lax.dot_general(lhs, x, _NT_DIMS, preferred_element_type=F32)

    def tiles(ref, unit0, j):
        return ref[pl.ds(unit0, 4), j].reshape(4 * T, DH)

    def over_keys(x, per_unit, op):
        red = jnp.max if op == "max" else jnp.sum
        x = red(x, axis=1, keepdims=True)
        if per_unit is True:
            return x
        fill = -jnp.inf if op == "max" else 0.0
        sec = lax.broadcasted_iota(jnp.int32, (8, 1), 0) >= 4
        lo = red(jnp.where(sec, fill, x), axis=0, keepdims=True)
        hi = red(jnp.where(sec, x, fill), axis=0, keepdims=True)
        whole = jnp.where(sec, hi, lo)
        return whole if per_unit is False else jnp.where(per_unit, x, whole)

    def tree(op, xs):
        while len(xs) > 1:
            xs = [op(xs[i], xs[i + 1]) for i in range(0, len(xs), 2)]
        return xs[0]

    def softmax(per_unit):
        s = [s_buf[j] * SCALE for j in range(NT)]
        m = over_keys(tree(jnp.maximum, s), per_unit, "max")
        e = [jnp.exp(x - m) for x in s]
        inv = 1.0 / over_keys(tree(jnp.add, e), per_unit, "sum")
        for j in range(NT):
            p_cur[j] = e[j] * inv

    def head_query(head):
        a = jnp.broadcast_to(qa[head >> 2, pl.ds(head & 3, 1), :], (8, DH))
        b = jnp.broadcast_to(qa[head >> 2, pl.ds(4 + (head & 3), 1), :], (8, DH))
        return blocks(jnp.where(second, b, a))

    def m_init():
        return jnp.zeros((DH + 16, DH), F32), jnp.zeros((8, DH), F32)

    def m_step(k_unit, v_unit, j, carry, loaded):
        acc, oacc = carry
        pk = blocks_f32(p_cur[j])
        v4 = tiles(vbuf, v_unit, j)
        k4 = tiles(pool, k_unit, j)
        p_row = jnp.concatenate([p_cur[j, pl.ds(4 + r, 1), :] for r in range(4)], axis=1)
        loaded()
        lhs = jnp.concatenate([v4.T.astype(F32) * p_row, pk, jnp.zeros_like(pk)], axis=0)
        acc = acc + jnp.dot(lhs.astype(BF16), k4, preferred_element_type=F32)
        oacc = oacc + jnp.dot(pk.astype(BF16), v4, preferred_element_type=F32)
        return acc, oacc

    def m_finish(carry):
        acc, oacc = carry
        o = jnp.sum(jnp.where(second, oacc, 0.0), axis=0, keepdims=True)
        kbar = jnp.sum(jnp.where(second, acc[DH:DH + 8], 0.0), axis=0, keepdims=True)
        o_col = jnp.broadcast_to(o, (DH, DH)).T
        return o, (acc[:DH] - o_col * kbar).astype(BF16)

    def cols(c):
        return pl.ds(pl.multiple_of(c * 1024, 1024), 1024)

    def rows8(v):
        return jnp.broadcast_to(v, (8, v.shape[1])).astype(BF16)

    def store_heads(dst, keep):
        def store(c, res):
            for k in range(2):
                v = res[:, 4 * k * DH:(4 * k + 1) * DH]
                for r in range(1, 4):
                    v = jnp.where(unit_of_row == r,
                                  res[:, (4 * k + r) * DH:(4 * k + r + 1) * DH], v)
                if keep is not None:
                    v = jnp.where(keep, dst[2 * c + k], v)
                dst[2 * c + k] = v
        return store

    def spread_heads(src, select):
        def spread(c):
            out = []
            for k in range(2):
                v = src[2 * c + k]
                if select is not None:
                    v = jnp.where(select, v, 0.0)
                out.append(blocks_f32(v))
            return jnp.concatenate(out, axis=1)
        return spread

    def to_heads_wq(v, wq, store):
        lhs = rows8(v)

        def body(c, _):
            w = wq[:, :, cols(c)].reshape(D, 1024)
            store(c, jnp.dot(lhs, w, preferred_element_type=F32))
        lax.fori_loop(0, 4, body, None)

    def to_heads_wo(v, wo, store):
        lhs = rows8(v)

        def body(c, _):
            store(c, lax.dot_general(lhs, wo[c], _NT_DIMS, preferred_element_type=F32))
        lax.fori_loop(0, 4, body, None)

    def from_heads_wo(spread, wo):
        def body(c, acc):
            return acc + jnp.dot(spread(c).astype(BF16), wo[c], preferred_element_type=F32)
        acc = lax.fori_loop(0, 4, body, jnp.zeros((8, D), F32))
        return jnp.sum(acc, axis=0, keepdims=True)

    def from_heads_wq(spread, wq):
        def body(c, acc):
            w = wq[:, :, cols(c)].reshape(D, 1024)
            return acc + lax.dot_general(spread(c).astype(BF16), w, _NT_DIMS,
                                         preferred_element_type=F32)
        acc = lax.fori_loop(0, 4, body, jnp.zeros((8, D), F32))
        return jnp.sum(acc, axis=0, keepdims=True)

    def layernorm(x, i):
        xc = x - jnp.mean(x, axis=1, keepdims=True)
        inv = 1.0 / jnp.sqrt(jnp.mean(xc * xc, axis=1, keepdims=True) + EPS)
        y = xc * inv
        vec[pl.ds(V_H + i, 1), :] = y
        inv_std[pl.ds(i, 1), :] = jnp.broadcast_to(inv, (1, T))
        return y

    def layernorm_bwd(dy, i):
        y = vec[pl.ds(V_H + i, 1), :]
        inv = inv_std[pl.ds(i, 1), pl.ds(0, 1)]
        return inv * (dy - jnp.mean(dy, axis=1, keepdims=True)
                      - y * jnp.mean(dy * y, axis=1, keepdims=True))

    def stage(a_now, a_next, work_a, b_now, b_next, work_b, carry=None, hook=None):
        def body(j, carry):
            if hook is not None:
                hook(j)
            a_now(j).wait(sem_a.at[j])
            if a_next is not None:
                a_next(j).start(sem_a.at[j])
            if work_a is not None:
                s_buf[j] = work_a(j)
            b_now(j).wait(sem_b.at[j])
            if b_next is not None:
                b_next(j).start(sem_b.at[j])
            if work_b is not None:
                carry = work_b(j, carry)
            return carry
        return lax.fori_loop(0, NT, body, carry)

    def scores(lhs, unit0):
        return lambda j: dot_keys(lhs, pool, unit0, j)

    def all_scores(lhs, unit0):
        def body(j, _):
            s_buf[j] = dot_keys(lhs, pool, unit0, j)
        lax.fori_loop(0, NT, body, None, unroll=4)

    wqa_a = lambda j: step_wq(wqa_hbm, wqa, 2 * j)
    wqa_b = lambda j: step_wq(wqa_hbm, wqa, 2 * j + 1)
    x_cp = pltpu.make_async_copy(x_hbm, x_io, sem_io.at[0])
    g_cp = pltpu.make_async_copy(g_hbm, g_io, sem_io.at[1])

    def first(j, _):
        wqa_a(j).start(sem_a.at[j])
        wqa_b(j).start(sem_b.at[j])
    lax.fori_loop(0, NT, first, None)
    x_cp.start()
    g_cp.start()
    for i, s in enumerate(A_SLOT):
        tab[TAB_A + i] = 4 * s
    for i, s in enumerate(KB_SLOT):
        tab[TAB_KB + i] = 4 * s
    for i, s in enumerate(STAGE_SLOT[:2 * NSTAGE]):
        tab[TAB_STAGE + i] = 4 * s
    zeros[...] = jnp.zeros(zeros.shape, BF16)
    oa[...] = jnp.zeros(oa.shape, F32)

    def head1(n):
        return (n + NRES) & (H - 1)

    slot0 = (NRES - H) % NSLOT

    def next_slot(s):
        return jnp.where(s == NSLOT - 1, 0, s + 1)

    def ka_steps(n, s):
        return lambda j: step_a(ka_hbm, head1(n), pool, 4 * s, j)

    def va_steps(n):
        return lambda j: step_a(va_hbm, head1(n), vbuf, 4 * head1(n), j)

    woa_lo = lambda j: step_wo(woa_hbm, woa, j)
    woa_hi = lambda j: step_wo(woa_hbm, woa, NT + j)
    wqb_a = lambda j: step_wq(wqb_hbm, wqb, 2 * j)
    wqb_b = lambda j: step_wq(wqb_hbm, wqb, 2 * j + 1)
    wob_lo = lambda j: step_wo(wob_hbm, wob, j)
    wob_hi = lambda j: step_wo(wob_hbm, wob, NT + j)

    stage(wqa_a, ka_steps(0, slot0), None, wqa_b, woa_lo, None)
    x_cp.wait()
    g_cp.wait()
    x0 = x_io[0].astype(F32)
    g4 = g_io[0].astype(F32)
    vec[pl.ds(V_G + 3, 1), :] = g4
    to_heads_wq(layernorm(x0, 0), wqa, store_heads(qa, None))

    stage(ka_steps(0, slot0), ka_steps(1, (slot0 + 1) % NSLOT), scores(head_query(head1(0)), 4 * slot0),
          woa_lo, va_steps(0), None)
    softmax(False)

    def head_first_use(n, s, a_now, a_next, b_next, has_next=True):
        s1 = next_slot(s)
        lhs = head_query(head1(n + 1)) if has_next else None

        def body(i, carry):
            j0, j1 = 2 * i, 2 * i + 1
            a_now(j0).wait(sem_a.at[j0])
            va_steps(n)(j0).wait(sem_b.at[j0])
            a_now(j1).wait(sem_a.at[j1])
            a_next(j0).start(sem_a.at[j0])
            va_steps(n)(j1).wait(sem_b.at[j1])
            b_next(j0).start(sem_b.at[j0])
            new_scores = []
            for j, start in ((j0, lambda: a_next(j1).start(sem_a.at[j1])),
                             (j1, lambda: b_next(j1).start(sem_b.at[j1]))):
                if has_next:
                    new_scores.append(dot_keys(lhs, pool, 4 * s1, j))
                carry = m_step(4 * s, 4 * head1(n), j, carry, start)
            for j, value in zip((j0, j1), new_scores):
                s_buf[j] = value
            return carry

        o, m = m_finish(lax.fori_loop(0, NT // 2, body, m_init()))
        oa[head1(n) >> 2, pl.ds(head1(n) & 3, 1), :] = o
        m1[head1(n)] = m
        if has_next:
            softmax(False)
        return s1

    def slot1(n):
        return (slot0 + n) % NSLOT

    lax.fori_loop(
        0, H - 2,
        lambda n, s: head_first_use(n, s, ka_steps(n + 1, next_slot(s)),
                                    ka_steps(n + 2, next_slot(next_slot(s))), va_steps(n + 1)),
        jnp.int32(slot0))
    head_first_use(H - 2, slot1(H - 2), ka_steps(H - 1, slot1(H - 1)), woa_hi, va_steps(H - 1))
    head_first_use(H - 1, slot1(H - 1), woa_hi, wqb_a, wqb_b, has_next=False)
    x1 = x0 + from_heads_wo(spread_heads(oa, ~second), woa)

    def kb_unit1(g):
        return 4 * (NRES + (g & 1))

    def kb_steps(g):
        return lambda j: step_b(kb_hbm, g, pool, kb_unit1(g), j)

    def vb_steps(g):
        return lambda j: step_b(vb_hbm, g, vbuf, VB0 + 4 * g, j)

    h2 = layernorm(x1, 1)
    stage(wqb_a, kb_steps(0), None, wqb_b, wob_lo, None)
    to_heads_wq(h2, wqb, store_heads(qb, None))
    stage(kb_steps(0), kb_steps(1), scores(blocks(qb[0]), kb_unit1(0)),
          wob_lo, vb_steps(0), None)
    softmax(True)

    def pv(g):
        def work(j, acc):
            return acc + jnp.dot(blocks(p_cur[j]), tiles(vbuf, VB0 + 4 * g, j),
                                 preferred_element_type=F32)
        return work

    def group_first_use(g, a_next):
        ob[g] = stage(kb_steps(g + 1), a_next, scores(blocks(qb[g + 1]), kb_unit1(g + 1)),
                      vb_steps(g), vb_steps(g + 1), pv(g), jnp.zeros((8, DH), F32))
        softmax(True)

    lax.fori_loop(0, NG - 2, lambda g, _: group_first_use(g, kb_steps(g + 2)), None)
    group_first_use(NG - 2, wob_hi)
    def early_zero(j):
        @pl.when(j == NT - LEAD_E2)
        def _():
            zero_fill(0, NZERO_FIRST, sem_zero.at[0], early=True)

    ob[NG - 1] = stage(wob_hi, None, None, vb_steps(NG - 1), None, pv(NG - 1),
                       jnp.zeros((8, DH), F32), early_zero)
    x2 = x1 + from_heads_wo(spread_heads(ob, ~second), wob)

    to_heads_wq(layernorm(x2, 2), wqa, store_heads(qa, ~second))

    def pm_unit(head):
        return jnp.where(head < 16, 4 * PM_SLOT[0], 4 * PM_SLOT[1])

    def pa_place(head):
        return pm_unit(head) + ((head >> 3) & 1), 2 * (head & 7)

    def p_tile(place, j):
        return place[0], place[1] + j // 8, pl.ds(16 * (j % 8), 16)

    def keep_p(place):
        for j in range(NT):
            pool[p_tile(place, j)] = pltpu.bitcast(p_cur[j], BF16)

    def load_p(place, j):
        return pltpu.bitcast(pool[p_tile(place, j)], F32)

    def slot_wait(unit0):
        slot = pool.at[pl.ds(unit0, 4)]
        pltpu.make_async_copy(slot, slot, sem_slot.at[unit0 >> 2]).wait()

    def reread_a(head, j):
        unit0 = tab[TAB_A + head]
        step_a(ka_hbm, head, pool, unit0, j).start(sem_slot.at[unit0 >> 2])

    def reread_b(g, j):
        unit0 = tab[TAB_KB + g]
        tail = (g == NG - 3) & (j >= NT - LEAD_E4)
        step_b(kb_hbm, g, pool, unit0, j).start(
            sem_slot.at[jnp.where(tail, NSLOT, unit0 >> 2)])

    def head_second_use(h, start_read):
        nxt = jnp.minimum(h + 1, H - 1)
        lhs = head_query(nxt)
        k_next, k_now = tab[TAB_A + nxt], tab[TAB_A + h]

        carry = m_init()
        for j in range(NT):
            s_buf[j] = dot_keys(lhs, pool, k_next, j)
            carry = m_step(k_now, 4 * h, j, carry, lambda: start_read(j))
        o, m = m_finish(carry)
        oa[h >> 2, pl.ds(4 + (h & 3), 1), :] = o
        keep_p(pa_place(h))
        pool[pm_unit(h) + 2, h & 15] = m
        softmax(False)

    zero_next = [NZERO_EARLY]

    def reserve_zero(n):
        lo = zero_next[0]
        zero_next[0] = min(lo + n, NZERO)
        return lo, zero_next[0]

    def more_zero(n):
        zero_fill(*reserve_zero(n), sem_zero.at[1])

    first_zero = reserve_zero(32)

    def reading_heads():
        pool[ZERO_UNIT, pl.ds(0, NG)] = jnp.zeros((NG, T, DH), BF16)
        zero_fill(0, NZERO_EARLY - LEAD_E3, sem_zero.at[0], early=True, wait=True)
        for k in range(CATCH_UP):
            lax.fori_loop(0, NT, lambda j, _: reread_a(NRES + k, j), None)
        first = FIRST_READER - CATCH_UP
        first_b = first + H - NRES

        def reader(reread, first_reader, base):
            def body(h, _):
                done = h - first - IN_FLIGHT
                pl.when(done >= 0)(lambda: slot_wait(tab[TAB_READ + jnp.maximum(done, 0)]))
                head_second_use(h, lambda j: reread(base + h - first_reader, j))
            return body

        lax.fori_loop(FIRST_READER, first_b,
                      reader(reread_a, FIRST_READER, NRES + CATCH_UP), None)
        lax.fori_loop(first_b, first_b + NG - 2, reader(reread_b, first_b, 0), None)
        for g in range(NG - 2 - IN_FLIGHT, NG - 3):
            slot_wait(4 * KB_SLOT[g])
        last = KB_SLOT[NG - 3]
        bulk = pool.at[pl.ds(4 * last, 4), pl.ds(0, NT - LEAD_E4)]
        tail = pool.at[pl.ds(4 * last, 4), pl.ds(NT - LEAD_E4, LEAD_E4)]
        pltpu.make_async_copy(bulk, bulk, sem_slot.at[last]).wait()
        zero_fill(*first_zero, sem_zero.at[1])
        pltpu.make_async_copy(tail, tail, sem_slot.at[NSLOT]).wait()

    freed_by = [h for h in range(H) if REFILL[h]]
    assert all(max(FIRST_READER - CATCH_UP + k, FIRST_READER) > h for k, h in enumerate(freed_by))
    end_readers = FIRST_READER - CATCH_UP + len(freed_by)
    assert end_readers <= H
    assert FIRST_READER - CATCH_UP + IN_FLIGHT < NRES

    def quiet_then_reading(i, _):
        lax.fori_loop(jnp.where(i == 0, 0, end_readers), jnp.where(i == 0, FIRST_READER, H),
                      lambda h, _: head_second_use(h, lambda j: None), None)
        pl.when(i == 0)(reading_heads)

    all_scores(head_query(0), 4 * A_SLOT[0])
    softmax(False)
    zero_fill(NZERO_FIRST, NZERO_EARLY - LEAD_E3, sem_zero.at[0], early=True)
    zero_fill(NZERO_EARLY - LEAD_E3, NZERO_EARLY, sem_zero.at[2], early=True)
    lax.fori_loop(0, 2, quiet_then_reading, None)
    more_zero(10)
    x3 = x2 + from_heads_wo(spread_heads(oa, second), woa)

    to_heads_wq(layernorm(x3, 3), wqb, store_heads(qb, ~second))
    to_heads_wo(g4, wob, store_heads(dob, None))

    def pb_place(g):
        return PB_UNIT, 2 * g

    def dscores(p, do8, o8, v_unit, stride):
        lhs = blocks(do8)
        delta = jnp.sum(do8.astype(BF16).astype(F32) * o8, axis=1, keepdims=True)
        return [p[j] * (dot_keys(lhs, vbuf, v_unit, j, stride) - delta) * SCALE
                for j in range(NT)]

    def dq_group(g):
        p = [load_p(pb_place(g), j) for j in range(NT)]
        ds = dscores(p, dob[g], ob[g], VB0 + 4 * g, 1)
        k_unit = tab[TAB_KB + g]
        dqb[g] = tree(jnp.add, [
            jnp.dot(blocks(ds[j]), tiles(pool, k_unit, j), preferred_element_type=F32)
            for j in range(NT)])

    group_zero = reserve_zero(6 * NG)[0]

    def group_second_use(g, _):
        zero_fill(group_zero + 6 * g, group_zero + 6 * (g + 1), sem_zero.at[1])
        all_scores(blocks(qb[g]), tab[TAB_KB + g])
        softmax(True)
        keep_p(pb_place(g))
        ob[g] = lax.fori_loop(0, NT, pv(g), jnp.zeros((8, DH), F32), unroll=4)
        dq_group(g)

    lax.fori_loop(0, NG, group_second_use, None)
    more_zero(24)
    x4 = x3 + from_heads_wo(spread_heads(ob, second), wob)
    x_io[0] = x4.astype(BF16)
    out_cp = pltpu.make_async_copy(x_io, out_hbm, sem_io.at[0])
    out_cp.start()

    def dq_heads(matrices, keep):
        def body(g, _):
            dq = SCALE * jnp.dot(blocks(doa[g]), matrices(g).reshape(4 * DH, DH),
                                 preferred_element_type=F32)
            dqa[g] = dq if keep is None else jnp.where(keep, dqa[g], dq)
        lax.fori_loop(0, NG, body, None, unroll=2)

    g3 = g4 + layernorm_bwd(from_heads_wq(spread_heads(dqb, second), wqb), 3)
    vec[pl.ds(V_G + 2, 1), :] = g3
    to_heads_wo(g3, woa, store_heads(doa, None))
    dq_heads(lambda g: pool[pm_unit(4 * g) + 2, pl.ds(4 * (g & 3), 4)], None)
    g2 = g3 + layernorm_bwd(from_heads_wq(spread_heads(dqa, second), wqa), 2)
    vec[pl.ds(V_G + 1, 1), :] = g2
    to_heads_wo(g2, wob, store_heads(dob, second))
    more_zero(24)
    lax.fori_loop(0, NG, lambda g, _: dq_group(g), None)
    more_zero(24)
    g1 = g2 + layernorm_bwd(from_heads_wq(spread_heads(dqb, ~second), wqb), 1)
    vec[pl.ds(V_G + 0, 1), :] = g1
    to_heads_wo(g1, woa, store_heads(doa, second))
    dq_heads(lambda g: m1[pl.ds(4 * g, 4)], second)
    g0 = g1 + layernorm_bwd(from_heads_wq(spread_heads(dqa, ~second), wqa), 0)
    g_io[0] = g0.astype(BF16)
    dx_cp = pltpu.make_async_copy(g_io, dx_hbm, sem_io.at[1])
    dx_cp.start()

    def both_uses(i):
        sec = lax.broadcasted_iota(jnp.int32, (8, D), 0) >= 4
        return jnp.where(sec, vec[pl.ds(i + 2, 1), :], vec[pl.ds(i, 1), :]).astype(BF16)

    def weight_grads(layer, wq, wo, dq_ref, o_ref):
        h_lhs, g_rhs = both_uses(V_H + layer), both_uses(V_G + layer)
        dq_spread, o_spread = spread_heads(dq_ref, None), spread_heads(o_ref, None)

        def body(c, _):
            dq, o = dq_spread(c), o_spread(c)
            for i in range(8):
                head = slice(i * DH, (i + 1) * DH)
                dq_i = dq[:, head].astype(BF16)
                head_cols = pl.ds(pl.multiple_of(c * 1024 + i * DH, DH), DH)
                for b in range(D // 128):
                    wq[b, :, head_cols] = lax.dot_general(
                        h_lhs[:, b * 128:(b + 1) * 128], dq_i, _TN_DIMS,
                        preferred_element_type=F32).astype(BF16)
                wo[c, head, :] = lax.dot_general(
                    o[:, head].astype(BF16), g_rhs, _TN_DIMS,
                    preferred_element_type=F32).astype(BF16)
        lax.fori_loop(0, 4, body, None)

    more_zero(NZERO)
    weight_grads(0, wqa, woa, dqa, oa)
    weight_grads(1, wqb, wob, dqb, ob)

    weights_out = ((wqa, dwqa_hbm, wq_piece, 5), (woa, dwoa_hbm, wo_piece, 4),
                   (wqb, dwqb_hbm, wq_piece, 5), (wob, dwob_hbm, wo_piece, 4))

    for i, (src, dst, piece, n) in enumerate(weights_out):
        lax.fori_loop(0, 2 * NT, lambda t, _: pltpu.make_async_copy(
            piece(src, t)(0, n), piece(dst, t)(0, n), sem_w.at[i]).start(), None)

    def outer_products(coef, vectors, unit0):
        lhs = jnp.concatenate(coef, axis=0).T.astype(BF16)
        zero = jnp.zeros_like(vectors)
        halves = (jnp.concatenate([vectors, zero], axis=0).astype(BF16),
                  jnp.concatenate([zero, vectors], axis=0).astype(BF16))
        zero16 = jnp.zeros((16, 4 * DH), BF16)
        for j in range(NT):
            rhs = jnp.concatenate(
                [halves[j % 2] if k == j // 2 else zero16 for k in range(NT // 2)], axis=0)
            res = jnp.dot(lhs, rhs, preferred_element_type=F32)
            for r in range(4):
                pool[unit0 + r, j] = res[:, r * DH:(r + 1) * DH].astype(BF16)

    def quarter_p(g, quarter, j):
        out = None
        for t in range(4):
            v = pltpu.roll(load_p(pa_place(4 * g + t), j), (t - quarter) & 7, 0)
            out = v if out is None else jnp.where(unit_of_row == t, v, out)
        return out

    def kv_grads(n, k):
        is_b = n < NG
        m = jnp.maximum(n - NG, 0)
        g, quarter = jnp.where(is_b, n, m >> 2), jnp.where(is_b, 3, m & 3)
        do8 = jnp.where(is_b, dob[g], doa[g])
        q8 = jnp.where(is_b, qb[g], qa[g])
        o8 = jnp.where(is_b, ob[g], oa[g])
        sk, sv = tab[TAB_STAGE + 2 * k], tab[TAB_STAGE + 2 * k + 1]

        @pl.when(n >= NSTAGE)
        def _():
            slot_wait(sk)
            slot_wait(sv)

        p = [jnp.where(is_b, load_p(pb_place(g), j), quarter_p(g, quarter, j)) for j in range(NT)]
        ds = dscores(p, do8, o8, jnp.where(is_b, VB0 + 4 * g, 16 * g + quarter),
                     jnp.where(is_b, 1, 4))
        outer_products(ds, blocks_f32(q8), sk)
        outer_products(p, blocks_f32(do8), sv)

        def issue(dk_hbm, dv_hbm):
            def body(j, _):
                for st, dst in ((sk, dk_hbm), (sv, dv_hbm)):
                    pltpu.make_async_copy(pool.at[pl.ds(st, 4), j], dst.at[g, :, quarter, j],
                                          sem_slot.at[st >> 2]).start()
            lax.fori_loop(0, NT, body, None, unroll=2)

        pl.when(is_b)(lambda: issue(dkb_hbm, dvb_hbm))
        pl.when(n >= NG)(lambda: issue(dka_hbm, dva_hbm))
        return jnp.where(k == NSTAGE - 1, 0, k + 1)

    lax.fori_loop(0, NG + H, kv_grads, jnp.int32(0))

    out_cp.wait()
    dx_cp.wait()
    zero_fill(NZERO_EARLY - LEAD_E3, NZERO_EARLY, sem_zero.at[2], early=True, wait=True)
    zero_fill(NZERO_EARLY, NZERO, sem_zero.at[1], wait=True)
    for i, (src, dst, _, _) in enumerate(weights_out):
        pltpu.make_async_copy(src, dst, sem_w.at[i]).wait()
    for s in STAGE_SLOT[:2 * NSTAGE]:
        slot_wait(4 * s)


@jax.jit
def pallas_interleave_layers__gqa_block_cached__sliding_block_cached__decode_kernel(
    A_x: jax.Array,
    A_k_cache: jax.Array,
    A_v_cache: jax.Array,
    A_wq: jax.Array,
    A_wo: jax.Array,
    B_x: jax.Array,
    B_k_cache: jax.Array,
    B_v_cache: jax.Array,
    B_wq: jax.Array,
    B_wo: jax.Array,
    grad_out: jax.Array,
):
    del B_x
    cache_shape = A_k_cache.shape
    a_view = (4 * H, NT, T, DH)
    b_view = (NG, 4, 4, NT, T, DH)
    wq_view = (5, 128, H * DH)
    wo_view = (4, 1024, D)

    def sds(shape):
        return jax.ShapeDtypeStruct(shape, BF16)

    io = pltpu.VMEM((1, 1, D), BF16)
    hbm = pl.BlockSpec(memory_space=pl.ANY)
    outs = pl.pallas_call(
        _kernel,
        out_shape=[sds((1, 1, D)), sds((1, 1, D)),
                   sds(b_view), sds(b_view), sds(wq_view), sds(wo_view),
                   sds(b_view), sds(b_view), sds(wq_view), sds(wo_view)],
        in_specs=[hbm] * 10,
        out_specs=[hbm] * 10,
        scratch_shapes=[
            pltpu.VMEM((5 * H, NT, T, DH), BF16),
            pltpu.VMEM(wq_view, BF16), pltpu.VMEM(wo_view, BF16),
            pltpu.VMEM(wq_view, BF16), pltpu.VMEM(wo_view, BF16),
            pltpu.VMEM((4 * NSLOT, NT, T, DH), BF16),
            pltpu.VMEM((H, DH, DH), BF16),
            pltpu.VMEM((4, T, DH), BF16),
            pltpu.VMEM((NT, 8, T), F32),
            pltpu.VMEM((NT, 8, T), F32),
            *[pltpu.VMEM((NG, 8, DH), F32)] * 8,
            pltpu.VMEM((8, D), F32), pltpu.VMEM((8, T), F32),
            io, io,
            pltpu.SMEM((TAB_SIZE,), jnp.int32),
            pltpu.SemaphoreType.DMA((NT,)), pltpu.SemaphoreType.DMA((NT,)),
            pltpu.SemaphoreType.DMA((NSLOT + 1,)), pltpu.SemaphoreType.DMA((3,)),
            pltpu.SemaphoreType.DMA((2,)), pltpu.SemaphoreType.DMA((4,)),
        ],
        compiler_params=pltpu.CompilerParams(vmem_limit_bytes=128 * 1024 * 1024),
    )(A_x, grad_out,
      A_k_cache.reshape(a_view), A_v_cache.reshape(a_view),
      A_wq.reshape(wq_view), A_wo.reshape(wo_view),
      B_k_cache.reshape(b_view), B_v_cache.reshape(b_view),
      B_wq.reshape(wq_view), B_wo.reshape(wo_view))
    out, dx, dka, dva, dwqa, dwoa, dkb, dvb, dwqb, dwob = outs
    return (out, dx,
            dka.reshape(cache_shape), dva.reshape(cache_shape),
            dwqa.reshape(A_wq.shape), dwoa.reshape(A_wo.shape),
            dkb.reshape(cache_shape), dvb.reshape(cache_shape),
            dwqb.reshape(B_wq.shape), dwob.reshape(B_wo.shape))
```

```python
import jax
import jax.numpy as jnp
from jax import lax
import jax.experimental.pallas as pl
import jax.experimental.pallas.tpu as pltpu

F32 = jnp.float32
BF16 = jnp.bfloat16

D = 640
H = 32
DH = 128
T = 128
NT = 16
NG = H // 4
SCALE = DH ** -0.5
EPS = 1e-5

NSLOT = 13
NRES = NSLOT - 2
VB0 = 4 * H

_NT_DIMS = (((1,), (1,)), ((), ()))
_TN_DIMS = (((0,), (0,)), ((), ()))


def _slot_plan():
    slot = list(range(NRES))
    kb_slot = [None] * NG
    kb_slot[NG - 2], kb_slot[NG - 1] = NRES, NRES + 1
    pm_slot = []
    refill = []
    todo = [("A", h) for h in range(NRES, H)] + [("B", g) for g in range(NG - 2)]
    for h in range(H):
        if h % 16 == 0:
            pm_slot.append(slot[h])
            refill.append(None)
        elif todo:
            kind, idx = todo.pop(0)
            refill.append((kind, idx))
            if kind == "A":
                slot.append(slot[h])
            else:
                kb_slot[idx] = slot[h]
        else:
            refill.append(None)
    assert not todo and len(slot) == H
    stage = [s for s in range(NSLOT) if s not in pm_slot]
    return slot, kb_slot, pm_slot, refill, stage


A_SLOT, KB_SLOT, PM_SLOT, REFILL, STAGE_SLOT = _slot_plan()
NSTAGE = len(STAGE_SLOT) // 2
ZERO_UNIT = 4 * PM_SLOT[0] + 3
PB_UNIT = 4 * PM_SLOT[1] + 3

NZERO = 3 * 4 * NT
NZERO_EARLY = 20
NZERO_FIRST = 12
FIRST_READER = 4
CATCH_UP = 1
IN_FLIGHT = 2
LEAD_ZERO = 1
LEAD_READ = 1
LEAD_WRITE = 4

TAB_A = 0
TAB_KB = TAB_A + H
TAB_READ = TAB_A + NRES
TAB_STAGE = TAB_KB + NG
TAB_SIZE = TAB_STAGE + 2 * NSTAGE

V_H, V_G = 0, 4


def _kernel(
    x_hbm, g_hbm, ka_hbm, va_hbm, wqa_hbm, woa_hbm, kb_hbm, vb_hbm, wqb_hbm, wob_hbm,
    out_hbm, dx_hbm, dka_hbm, dva_hbm, dwqa_hbm, dwoa_hbm, dkb_hbm, dvb_hbm, dwqb_hbm, dwob_hbm,
    vbuf, wqa, woa, wqb, wob, pool, m1, zeros, s_buf, p_cur,
    qa, oa, doa, dqa, qb, ob, dob, dqb, vec, inv_std,
    x_io, g_io, tab,
    sem_a, sem_b, sem_slot, sem_zero, sem_io, sem_w,
):
    row8 = lax.broadcasted_iota(jnp.int32, (8, T), 0)
    unit_of_row = row8 & 3
    second = row8 >= 4

    class Step:
        def __init__(self, src, dst, n=4):
            self.src, self.dst, self.n = src, dst, n

        def start(self, sem):
            n = self.n
            pltpu.make_async_copy(self.src(0, n - 1), self.dst(0, n - 1), sem).start(priority=1)
            pltpu.make_async_copy(self.src(n - 1, 1), self.dst(n - 1, 1), sem).start(priority=0)

        def wait(self, sem):
            pltpu.make_async_copy(self.src(0, self.n), self.dst(0, self.n), sem).wait()

    def step_a(src, head, dst, unit0, j):
        return Step(lambda r, n: src.at[pl.ds(4 * head + r, n), j],
                    lambda r, n: dst.at[pl.ds(unit0 + r, n), j])

    def step_b(src, group, dst, unit0, j):
        return Step(lambda r, n: src.at[group, pl.ds(r, n), 3, j],
                    lambda r, n: dst.at[pl.ds(unit0 + r, n), j])

    def wq_piece(ref, t):
        rr = pl.ds(pl.multiple_of((t >> 1) * 8, 8), 8)
        cc = pl.ds(pl.multiple_of((t & 1) * 2048, 2048), 2048)
        return lambda r, n: ref.at[pl.ds(r, n), rr, cc]

    def wo_piece(ref, t):
        rr = pl.ds(pl.multiple_of(t * 32, 32), 32)
        return lambda r, n: ref.at[pl.ds(r, n), rr]

    def step_wq(src, dst, t):
        return Step(wq_piece(src, t), wq_piece(dst, t), 5)

    def step_wo(src, dst, t):
        return Step(wo_piece(src, t), wo_piece(dst, t))

    def zero_fill(lo, hi, sem, early=False, wait=False):
        def body(i, _):
            j, head, quarter = i & (NT - 1), (i >> 4) & 3, i >> 6
            for dst in (dkb_hbm, dvb_hbm):
                if early:
                    copies = [(zeros, dst.at[pl.ds(4 * k, 4), head, quarter, j]) for k in range(2)]
                else:
                    copies = [(pool.at[ZERO_UNIT, pl.ds(0, NG)], dst.at[:, head, quarter, j])]
                for src, dst_block in copies:
                    cp = pltpu.make_async_copy(src, dst_block, sem)
                    cp.wait() if wait else cp.start()

        lax.fori_loop(lo, hi, body, None)

    def blocks_f32(v8):
        return jnp.concatenate(
            [jnp.where(unit_of_row == r, v8, 0.0) for r in range(4)], axis=1)

    def blocks(v8):
        return blocks_f32(v8).astype(BF16)

    def dot_keys(lhs, ref, unit0, j, stride=1):
        x = jnp.concatenate([ref[unit0 + r * stride, j] for r in range(4)], axis=1)
        return lax.dot_general(lhs, x, _NT_DIMS, preferred_element_type=F32)

    def tiles(ref, unit0, j):
        return ref[pl.ds(unit0, 4), j].reshape(4 * T, DH)

    def over_keys(x, per_unit, op):
        red = jnp.max if op == "max" else jnp.sum
        x = red(x, axis=1, keepdims=True)
        if per_unit:
            return x
        fill = -jnp.inf if op == "max" else 0.0
        sec = lax.broadcasted_iota(jnp.int32, (8, 1), 0) >= 4
        lo = red(jnp.where(sec, fill, x), axis=0, keepdims=True)
        hi = red(jnp.where(sec, x, fill), axis=0, keepdims=True)
        return jnp.where(sec, hi, lo)

    def tree(op, xs):
        while len(xs) > 1:
            xs = [op(xs[i], xs[i + 1]) for i in range(0, len(xs), 2)]
        return xs[0]

    def softmax(per_unit):
        s = [s_buf[j] * SCALE for j in range(NT)]
        m = over_keys(tree(jnp.maximum, s), per_unit, "max")
        e = [jnp.exp(x - m) for x in s]
        inv = 1.0 / over_keys(tree(jnp.add, e), per_unit, "sum")
        for j in range(NT):
            p_cur[j] = e[j] * inv

    def head_query(head):
        a = jnp.broadcast_to(qa[head >> 2, pl.ds(head & 3, 1), :], (8, DH))
        b = jnp.broadcast_to(qa[head >> 2, pl.ds(4 + (head & 3), 1), :], (8, DH))
        return blocks(jnp.where(second, b, a))

    def m_init():
        return jnp.zeros((DH + 16, DH), F32), jnp.zeros((8, DH), F32)

    def m_step(k_unit, v_unit, j, carry, loaded):
        acc, oacc = carry
        pk = blocks_f32(p_cur[j])
        v4 = tiles(vbuf, v_unit, j)
        k4 = tiles(pool, k_unit, j)
        p_row = jnp.concatenate([p_cur[j, pl.ds(4 + r, 1), :] for r in range(4)], axis=1)
        loaded()
        lhs = jnp.concatenate([v4.T.astype(F32) * p_row, pk, jnp.zeros_like(pk)], axis=0)
        acc = acc + jnp.dot(lhs.astype(BF16), k4, preferred_element_type=F32)
        oacc = oacc + jnp.dot(pk.astype(BF16), v4, preferred_element_type=F32)
        return acc, oacc

    def m_finish(carry):
        acc, oacc = carry
        o = jnp.sum(jnp.where(second, oacc, 0.0), axis=0, keepdims=True)
        kbar = jnp.sum(jnp.where(second, acc[DH:DH + 8], 0.0), axis=0, keepdims=True)
        o_col = jnp.broadcast_to(o, (DH, DH)).T
        return o, (acc[:DH] - o_col * kbar).astype(BF16)

    def cols(c):
        return pl.ds(pl.multiple_of(c * 1024, 1024), 1024)

    def rows8(v):
        return jnp.broadcast_to(v, (8, v.shape[1])).astype(BF16)

    def store_heads(dst, keep):
        def store(c, res):
            for k in range(2):
                v = res[:, 4 * k * DH:(4 * k + 1) * DH]
                for r in range(1, 4):
                    v = jnp.where(unit_of_row == r,
                                  res[:, (4 * k + r) * DH:(4 * k + r + 1) * DH], v)
                if keep is not None:
                    v = jnp.where(keep, dst[2 * c + k], v)
                dst[2 * c + k] = v
        return store

    def spread_heads(src, select):
        def spread(c):
            out = []
            for k in range(2):
                v = src[2 * c + k]
                if select is not None:
                    v = jnp.where(select, v, 0.0)
                out.append(blocks_f32(v))
            return jnp.concatenate(out, axis=1)
        return spread

    def to_heads_wq(v, wq, store):
        lhs = rows8(v)

        def body(c, _):
            w = wq[:, :, cols(c)].reshape(D, 1024)
            store(c, jnp.dot(lhs, w, preferred_element_type=F32))
        lax.fori_loop(0, 4, body, None)

    def to_heads_wo(v, wo, store):
        lhs = rows8(v)

        def body(c, _):
            store(c, lax.dot_general(lhs, wo[c], _NT_DIMS, preferred_element_type=F32))
        lax.fori_loop(0, 4, body, None)

    def from_heads_wo(spread, wo):
        def body(c, acc):
            return acc + jnp.dot(spread(c).astype(BF16), wo[c], preferred_element_type=F32)
        acc = lax.fori_loop(0, 4, body, jnp.zeros((8, D), F32))
        return jnp.sum(acc, axis=0, keepdims=True)

    def from_heads_wq(spread, wq):
        def body(c, acc):
            w = wq[:, :, cols(c)].reshape(D, 1024)
            return acc + lax.dot_general(spread(c).astype(BF16), w, _NT_DIMS,
                                         preferred_element_type=F32)
        acc = lax.fori_loop(0, 4, body, jnp.zeros((8, D), F32))
        return jnp.sum(acc, axis=0, keepdims=True)

    def layernorm(x, i):
        xc = x - jnp.mean(x, axis=1, keepdims=True)
        inv = 1.0 / jnp.sqrt(jnp.mean(xc * xc, axis=1, keepdims=True) + EPS)
        y = xc * inv
        vec[pl.ds(V_H + i, 1), :] = y
        inv_std[pl.ds(i, 1), :] = jnp.broadcast_to(inv, (1, T))
        return y

    def layernorm_bwd(dy, i):
        y = vec[pl.ds(V_H + i, 1), :]
        inv = inv_std[pl.ds(i, 1), pl.ds(0, 1)]
        return inv * (dy - jnp.mean(dy, axis=1, keepdims=True)
                      - y * jnp.mean(dy * y, axis=1, keepdims=True))

    def stage(a_now, a_next, work_a, b_now, b_next, work_b, carry=None, hook=None):
        def body(j, carry):
            if hook is not None:
                hook(j)
            a_now(j).wait(sem_a.at[j])
            if a_next is not None:
                a_next(j).start(sem_a.at[j])
            if work_a is not None:
                s_buf[j] = work_a(j)
            b_now(j).wait(sem_b.at[j])
            if b_next is not None:
                b_next(j).start(sem_b.at[j])
            if work_b is not None:
                carry = work_b(j, carry)
            return carry
        return lax.fori_loop(0, NT, body, carry)

    def scores(lhs, unit0):
        return lambda j: dot_keys(lhs, pool, unit0, j)

    def all_scores(lhs, unit0):
        def body(j, _):
            s_buf[j] = dot_keys(lhs, pool, unit0, j)
        lax.fori_loop(0, NT, body, None, unroll=4)

    wqa_a = lambda j: step_wq(wqa_hbm, wqa, 2 * j)
    wqa_b = lambda j: step_wq(wqa_hbm, wqa, 2 * j + 1)
    x_cp = pltpu.make_async_copy(x_hbm, x_io, sem_io.at[0])
    g_cp = pltpu.make_async_copy(g_hbm, g_io, sem_io.at[1])

    def first(j, _):
        wqa_a(j).start(sem_a.at[j])
        wqa_b(j).start(sem_b.at[j])
    lax.fori_loop(0, NT, first, None)
    x_cp.start()
    g_cp.start()
    for i, s in enumerate(A_SLOT):
        tab[TAB_A + i] = 4 * s
    for i, s in enumerate(KB_SLOT):
        tab[TAB_KB + i] = 4 * s
    for i, s in enumerate(STAGE_SLOT[:2 * NSTAGE]):
        tab[TAB_STAGE + i] = 4 * s
    zeros[...] = jnp.zeros(zeros.shape, BF16)
    oa[...] = jnp.zeros(oa.shape, F32)

    def head1(n):
        return (n + NRES) & (H - 1)

    slot0 = (NRES - H) % NSLOT

    def slot1(n):
        return (slot0 + n) % NSLOT

    def next_slot(s):
        return jnp.where(s == NSLOT - 1, 0, s + 1)

    def ka_steps(n, s):
        return lambda j: step_a(ka_hbm, head1(n), pool, 4 * s, j)

    def va_steps(n):
        return lambda j: step_a(va_hbm, head1(n), vbuf, 4 * head1(n), j)

    woa_lo = lambda j: step_wo(woa_hbm, woa, j)
    woa_hi = lambda j: step_wo(woa_hbm, woa, NT + j)
    wqb_a = lambda j: step_wq(wqb_hbm, wqb, 2 * j)
    wqb_b = lambda j: step_wq(wqb_hbm, wqb, 2 * j + 1)
    wob_lo = lambda j: step_wo(wob_hbm, wob, j)
    wob_hi = lambda j: step_wo(wob_hbm, wob, NT + j)

    stage(wqa_a, ka_steps(0, slot0), None, wqa_b, woa_lo, None)
    x_cp.wait()
    g_cp.wait()
    x0 = x_io[0].astype(F32)
    g4 = g_io[0].astype(F32)
    vec[pl.ds(V_G + 3, 1), :] = g4
    to_heads_wq(layernorm(x0, 0), wqa, store_heads(qa, None))

    stage(ka_steps(0, slot0), ka_steps(1, slot1(1)), scores(head_query(head1(0)), 4 * slot0),
          woa_lo, va_steps(0), None)
    softmax(False)

    def head_first_use(n, s, a_now, a_next, b_next, has_next=True):
        s1 = next_slot(s)
        lhs = head_query(head1(n + 1)) if has_next else None

        def body(i, carry):
            j0, j1 = 2 * i, 2 * i + 1
            a_now(j0).wait(sem_a.at[j0])
            va_steps(n)(j0).wait(sem_b.at[j0])
            a_now(j1).wait(sem_a.at[j1])
            a_next(j0).start(sem_a.at[j0])
            va_steps(n)(j1).wait(sem_b.at[j1])
            b_next(j0).start(sem_b.at[j0])
            new_scores = []
            for j, start in ((j0, lambda: a_next(j1).start(sem_a.at[j1])),
                             (j1, lambda: b_next(j1).start(sem_b.at[j1]))):
                if has_next:
                    new_scores.append(dot_keys(lhs, pool, 4 * s1, j))
                carry = m_step(4 * s, 4 * head1(n), j, carry, start)
            for j, value in zip((j0, j1), new_scores):
                s_buf[j] = value
            return carry

        o, m = m_finish(lax.fori_loop(0, NT // 2, body, m_init()))
        oa[head1(n) >> 2, pl.ds(head1(n) & 3, 1), :] = o
        m1[head1(n)] = m
        if has_next:
            softmax(False)
        return s1

    lax.fori_loop(
        0, H - 2,
        lambda n, s: head_first_use(n, s, ka_steps(n + 1, next_slot(s)),
                                    ka_steps(n + 2, next_slot(next_slot(s))), va_steps(n + 1)),
        jnp.int32(slot0))
    head_first_use(H - 2, slot1(H - 2), ka_steps(H - 1, slot1(H - 1)), woa_hi, va_steps(H - 1))
    head_first_use(H - 1, slot1(H - 1), woa_hi, wqb_a, wqb_b, has_next=False)
    x1 = x0 + from_heads_wo(spread_heads(oa, ~second), woa)

    def kb_unit1(g):
        return 4 * (NRES + (g & 1))

    def kb_steps(g):
        return lambda j: step_b(kb_hbm, g, pool, kb_unit1(g), j)

    def vb_steps(g):
        return lambda j: step_b(vb_hbm, g, vbuf, VB0 + 4 * g, j)

    h2 = layernorm(x1, 1)
    stage(wqb_a, kb_steps(0), None, wqb_b, wob_lo, None)
    to_heads_wq(h2, wqb, store_heads(qb, None))
    stage(kb_steps(0), kb_steps(1), scores(blocks(qb[0]), kb_unit1(0)),
          wob_lo, vb_steps(0), None)
    softmax(True)

    def pv(g):
        def work(j, acc):
            return acc + jnp.dot(blocks(p_cur[j]), tiles(vbuf, VB0 + 4 * g, j),
                                 preferred_element_type=F32)
        return work

    def group_first_use(g, a_next):
        ob[g] = stage(kb_steps(g + 1), a_next, scores(blocks(qb[g + 1]), kb_unit1(g + 1)),
                      vb_steps(g), vb_steps(g + 1), pv(g), jnp.zeros((8, DH), F32))
        softmax(True)

    lax.fori_loop(0, NG - 2, lambda g, _: group_first_use(g, kb_steps(g + 2)), None)
    group_first_use(NG - 2, wob_hi)

    def early_zero(j):
        @pl.when(j == NT - LEAD_ZERO)
        def _():
            zero_fill(0, NZERO_FIRST, sem_zero.at[0], early=True)

    ob[NG - 1] = stage(wob_hi, None, None, vb_steps(NG - 1), None, pv(NG - 1),
                       jnp.zeros((8, DH), F32), early_zero)
    x2 = x1 + from_heads_wo(spread_heads(ob, ~second), wob)

    to_heads_wq(layernorm(x2, 2), wqa, store_heads(qa, ~second))

    def pm_unit(head):
        return jnp.where(head < 16, 4 * PM_SLOT[0], 4 * PM_SLOT[1])

    def pa_place(head):
        return pm_unit(head) + ((head >> 3) & 1), 2 * (head & 7)

    def p_tile(place, j):
        return place[0], place[1] + j // 8, pl.ds(16 * (j % 8), 16)

    def keep_p(place):
        for j in range(NT):
            pool[p_tile(place, j)] = pltpu.bitcast(p_cur[j], BF16)

    def load_p(place, j):
        return pltpu.bitcast(pool[p_tile(place, j)], F32)

    def slot_wait(unit0):
        slot = pool.at[pl.ds(unit0, 4)]
        pltpu.make_async_copy(slot, slot, sem_slot.at[unit0 >> 2]).wait()

    def reread_a(head, j):
        unit0 = tab[TAB_A + head]
        step_a(ka_hbm, head, pool, unit0, j).start(sem_slot.at[unit0 >> 2])

    def reread_b(g, j):
        unit0 = tab[TAB_KB + g]
        tail = (g == NG - 3) & (j >= NT - LEAD_WRITE)
        step_b(kb_hbm, g, pool, unit0, j).start(
            sem_slot.at[jnp.where(tail, NSLOT, unit0 >> 2)])

    def head_second_use(h, start_read):
        nxt = jnp.minimum(h + 1, H - 1)
        lhs = head_query(nxt)
        k_next, k_now = tab[TAB_A + nxt], tab[TAB_A + h]

        carry = m_init()
        for j in range(NT):
            s_buf[j] = dot_keys(lhs, pool, k_next, j)
            carry = m_step(k_now, 4 * h, j, carry, lambda: start_read(j))
        o, m = m_finish(carry)
        oa[h >> 2, pl.ds(4 + (h & 3), 1), :] = o
        keep_p(pa_place(h))
        pool[pm_unit(h) + 2, h & 15] = m
        softmax(False)

    zero_next = [NZERO_EARLY]

    def reserve_zero(n):
        lo = zero_next[0]
        zero_next[0] = min(lo + n, NZERO)
        return lo, zero_next[0]

    def more_zero(n):
        zero_fill(*reserve_zero(n), sem_zero.at[1])

    first_zero = reserve_zero(32)

    def reading_heads():
        pool[ZERO_UNIT, pl.ds(0, NG)] = jnp.zeros((NG, T, DH), BF16)
        zero_fill(0, NZERO_EARLY - LEAD_READ, sem_zero.at[0], early=True, wait=True)
        for k in range(CATCH_UP):
            lax.fori_loop(0, NT, lambda j, _: reread_a(NRES + k, j), None)
        first = FIRST_READER - CATCH_UP
        first_b = first + H - NRES

        def reader(reread, first_reader, base):
            def body(h, _):
                done = h - first - IN_FLIGHT
                pl.when(done >= 0)(lambda: slot_wait(tab[TAB_READ + jnp.maximum(done, 0)]))
                head_second_use(h, lambda j: reread(base + h - first_reader, j))
            return body

        lax.fori_loop(FIRST_READER, first_b,
                      reader(reread_a, FIRST_READER, NRES + CATCH_UP), None)
        lax.fori_loop(first_b, first_b + NG - 2, reader(reread_b, first_b, 0), None)
        for g in range(NG - 2 - IN_FLIGHT, NG - 3):
            slot_wait(4 * KB_SLOT[g])
        last = KB_SLOT[NG - 3]
        bulk = pool.at[pl.ds(4 * last, 4), pl.ds(0, NT - LEAD_WRITE)]
        tail = pool.at[pl.ds(4 * last, 4), pl.ds(NT - LEAD_WRITE, LEAD_WRITE)]
        pltpu.make_async_copy(bulk, bulk, sem_slot.at[last]).wait()
        zero_fill(*first_zero, sem_zero.at[1])
        pltpu.make_async_copy(tail, tail, sem_slot.at[NSLOT]).wait()

    freed_by = [h for h in range(H) if REFILL[h]]
    assert all(max(FIRST_READER - CATCH_UP + k, FIRST_READER) > h for k, h in enumerate(freed_by))
    end_readers = FIRST_READER - CATCH_UP + len(freed_by)
    assert end_readers <= H
    assert FIRST_READER - CATCH_UP + IN_FLIGHT < NRES

    def quiet_then_reading(i, _):
        lax.fori_loop(jnp.where(i == 0, 0, end_readers), jnp.where(i == 0, FIRST_READER, H),
                      lambda h, _: head_second_use(h, lambda j: None), None)
        pl.when(i == 0)(reading_heads)

    all_scores(head_query(0), 4 * A_SLOT[0])
    softmax(False)
    zero_fill(NZERO_FIRST, NZERO_EARLY - LEAD_READ, sem_zero.at[0], early=True)
    zero_fill(NZERO_EARLY - LEAD_READ, NZERO_EARLY, sem_zero.at[2], early=True)
    lax.fori_loop(0, 2, quiet_then_reading, None)
    more_zero(10)
    x3 = x2 + from_heads_wo(spread_heads(oa, second), woa)

    to_heads_wq(layernorm(x3, 3), wqb, store_heads(qb, ~second))
    to_heads_wo(g4, wob, store_heads(dob, None))

    def pb_place(g):
        return PB_UNIT, 2 * g

    def dscores(p, do8, o8, v_unit, stride):
        lhs = blocks(do8)
        delta = jnp.sum(do8.astype(BF16).astype(F32) * o8, axis=1, keepdims=True)
        return [p[j] * (dot_keys(lhs, vbuf, v_unit, j, stride) - delta) * SCALE
                for j in range(NT)]

    def dq_group(g):
        p = [load_p(pb_place(g), j) for j in range(NT)]
        ds = dscores(p, dob[g], ob[g], VB0 + 4 * g, 1)
        k_unit = tab[TAB_KB + g]
        dqb[g] = tree(jnp.add, [
            jnp.dot(blocks(ds[j]), tiles(pool, k_unit, j), preferred_element_type=F32)
            for j in range(NT)])

    group_zero = reserve_zero(6 * NG)[0]

    def group_second_use(g, _):
        zero_fill(group_zero + 6 * g, group_zero + 6 * (g + 1), sem_zero.at[1])
        all_scores(blocks(qb[g]), tab[TAB_KB + g])
        softmax(True)
        keep_p(pb_place(g))
        ob[g] = lax.fori_loop(0, NT, pv(g), jnp.zeros((8, DH), F32), unroll=4)
        dq_group(g)

    lax.fori_loop(0, NG, group_second_use, None)
    more_zero(24)
    x4 = x3 + from_heads_wo(spread_heads(ob, second), wob)
    x_io[0] = x4.astype(BF16)
    out_cp = pltpu.make_async_copy(x_io, out_hbm, sem_io.at[0])
    out_cp.start()

    def dq_heads(matrices, keep):
        def body(g, _):
            dq = SCALE * jnp.dot(blocks(doa[g]), matrices(g).reshape(4 * DH, DH),
                                 preferred_element_type=F32)
            dqa[g] = dq if keep is None else jnp.where(keep, dqa[g], dq)
        lax.fori_loop(0, NG, body, None, unroll=2)

    g3 = g4 + layernorm_bwd(from_heads_wq(spread_heads(dqb, second), wqb), 3)
    vec[pl.ds(V_G + 2, 1), :] = g3
    to_heads_wo(g3, woa, store_heads(doa, None))
    dq_heads(lambda g: pool[pm_unit(4 * g) + 2, pl.ds(4 * (g & 3), 4)], None)
    g2 = g3 + layernorm_bwd(from_heads_wq(spread_heads(dqa, second), wqa), 2)
    vec[pl.ds(V_G + 1, 1), :] = g2
    to_heads_wo(g2, wob, store_heads(dob, second))
    more_zero(24)
    lax.fori_loop(0, NG, lambda g, _: dq_group(g), None)
    more_zero(24)
    g1 = g2 + layernorm_bwd(from_heads_wq(spread_heads(dqb, ~second), wqb), 1)
    vec[pl.ds(V_G + 0, 1), :] = g1
    to_heads_wo(g1, woa, store_heads(doa, second))
    dq_heads(lambda g: m1[pl.ds(4 * g, 4)], second)
    g0 = g1 + layernorm_bwd(from_heads_wq(spread_heads(dqa, ~second), wqa), 0)
    g_io[0] = g0.astype(BF16)
    dx_cp = pltpu.make_async_copy(g_io, dx_hbm, sem_io.at[1])
    dx_cp.start()

    def both_uses(i):
        sec = lax.broadcasted_iota(jnp.int32, (8, D), 0) >= 4
        return jnp.where(sec, vec[pl.ds(i + 2, 1), :], vec[pl.ds(i, 1), :]).astype(BF16)

    def weight_grads(layer, wq, wo, dq_ref, o_ref):
        h_lhs, g_rhs = both_uses(V_H + layer), both_uses(V_G + layer)
        dq_spread, o_spread = spread_heads(dq_ref, None), spread_heads(o_ref, None)

        def body(c, _):
            dq, o = dq_spread(c), o_spread(c)
            for i in range(8):
                head = slice(i * DH, (i + 1) * DH)
                dq_i = dq[:, head].astype(BF16)
                head_cols = pl.ds(pl.multiple_of(c * 1024 + i * DH, DH), DH)
                for b in range(D // 128):
                    wq[b, :, head_cols] = lax.dot_general(
                        h_lhs[:, b * 128:(b + 1) * 128], dq_i, _TN_DIMS,
                        preferred_element_type=F32).astype(BF16)
                wo[c, head, :] = lax.dot_general(
                    o[:, head].astype(BF16), g_rhs, _TN_DIMS,
                    preferred_element_type=F32).astype(BF16)
        lax.fori_loop(0, 4, body, None)

    more_zero(NZERO)
    weight_grads(0, wqa, woa, dqa, oa)
    weight_grads(1, wqb, wob, dqb, ob)

    weights_out = ((wqa, dwqa_hbm, wq_piece, 5), (woa, dwoa_hbm, wo_piece, 4),
                   (wqb, dwqb_hbm, wq_piece, 5), (wob, dwob_hbm, wo_piece, 4))

    for i, (src, dst, piece, n) in enumerate(weights_out):
        lax.fori_loop(0, 2 * NT, lambda t, _: pltpu.make_async_copy(
            piece(src, t)(0, n), piece(dst, t)(0, n), sem_w.at[i]).start(), None)

    def outer_products(coef, vectors, unit0):
        lhs = jnp.concatenate(coef, axis=0).T.astype(BF16)
        zero = jnp.zeros_like(vectors)
        halves = (jnp.concatenate([vectors, zero], axis=0).astype(BF16),
                  jnp.concatenate([zero, vectors], axis=0).astype(BF16))
        zero16 = jnp.zeros((16, 4 * DH), BF16)
        for j in range(NT):
            rhs = jnp.concatenate(
                [halves[j % 2] if k == j // 2 else zero16 for k in range(NT // 2)], axis=0)
            res = jnp.dot(lhs, rhs, preferred_element_type=F32)
            for r in range(4):
                pool[unit0 + r, j] = res[:, r * DH:(r + 1) * DH].astype(BF16)

    def quarter_p(g, quarter, j):
        out = None
        for t in range(4):
            v = pltpu.roll(load_p(pa_place(4 * g + t), j), (t - quarter) & 7, 0)
            out = v if out is None else jnp.where(unit_of_row == t, v, out)
        return out

    def kv_grads(n, k):
        is_b = n < NG
        m = jnp.maximum(n - NG, 0)
        g, quarter = jnp.where(is_b, n, m >> 2), jnp.where(is_b, 3, m & 3)
        do8 = jnp.where(is_b, dob[g], doa[g])
        q8 = jnp.where(is_b, qb[g], qa[g])
        o8 = jnp.where(is_b, ob[g], oa[g])
        sk, sv = tab[TAB_STAGE + 2 * k], tab[TAB_STAGE + 2 * k + 1]

        @pl.when(n >= NSTAGE)
        def _():
            slot_wait(sk)
            slot_wait(sv)

        p = [jnp.where(is_b, load_p(pb_place(g), j), quarter_p(g, quarter, j)) for j in range(NT)]
        ds = dscores(p, do8, o8, jnp.where(is_b, VB0 + 4 * g, 16 * g + quarter),
                     jnp.where(is_b, 1, 4))
        outer_products(ds, blocks_f32(q8), sk)
        outer_products(p, blocks_f32(do8), sv)

        def issue(dk_hbm, dv_hbm):
            def body(j, _):
                for st, dst in ((sk, dk_hbm), (sv, dv_hbm)):
                    pltpu.make_async_copy(pool.at[pl.ds(st, 4), j], dst.at[g, :, quarter, j],
                                          sem_slot.at[st >> 2]).start()
            lax.fori_loop(0, NT, body, None, unroll=2)

        pl.when(is_b)(lambda: issue(dkb_hbm, dvb_hbm))
        pl.when(n >= NG)(lambda: issue(dka_hbm, dva_hbm))
        return jnp.where(k == NSTAGE - 1, 0, k + 1)

    lax.fori_loop(0, NG + H, kv_grads, jnp.int32(0))

    out_cp.wait()
    dx_cp.wait()
    zero_fill(NZERO_EARLY - LEAD_READ, NZERO_EARLY, sem_zero.at[2], early=True, wait=True)
    zero_fill(NZERO_EARLY, NZERO, sem_zero.at[1], wait=True)
    for i, (src, dst, _, _) in enumerate(weights_out):
        pltpu.make_async_copy(src, dst, sem_w.at[i]).wait()
    for s in STAGE_SLOT[:2 * NSTAGE]:
        slot_wait(4 * s)


@jax.jit
def pallas_interleave_layers__gqa_block_cached__sliding_block_cached__decode_kernel(
    A_x: jax.Array,
    A_k_cache: jax.Array,
    A_v_cache: jax.Array,
    A_wq: jax.Array,
    A_wo: jax.Array,
    B_x: jax.Array,
    B_k_cache: jax.Array,
    B_v_cache: jax.Array,
    B_wq: jax.Array,
    B_wo: jax.Array,
    grad_out: jax.Array,
):
    del B_x
    cache_shape = A_k_cache.shape
    a_view = (4 * H, NT, T, DH)
    b_view = (NG, 4, 4, NT, T, DH)
    wq_view = (5, 128, H * DH)
    wo_view = (4, 1024, D)

    def sds(shape):
        return jax.ShapeDtypeStruct(shape, BF16)

    io = pltpu.VMEM((1, 1, D), BF16)
    hbm = pl.BlockSpec(memory_space=pl.ANY)
    outs = pl.pallas_call(
        _kernel,
        out_shape=[sds((1, 1, D)), sds((1, 1, D)),
                   sds(b_view), sds(b_view), sds(wq_view), sds(wo_view),
                   sds(b_view), sds(b_view), sds(wq_view), sds(wo_view)],
        in_specs=[hbm] * 10,
        out_specs=[hbm] * 10,
        scratch_shapes=[
            pltpu.VMEM((5 * H, NT, T, DH), BF16),
            pltpu.VMEM(wq_view, BF16), pltpu.VMEM(wo_view, BF16),
            pltpu.VMEM(wq_view, BF16), pltpu.VMEM(wo_view, BF16),
            pltpu.VMEM((4 * NSLOT, NT, T, DH), BF16),
            pltpu.VMEM((H, DH, DH), BF16),
            pltpu.VMEM((4, T, DH), BF16),
            pltpu.VMEM((NT, 8, T), F32),
            pltpu.VMEM((NT, 8, T), F32),
            *[pltpu.VMEM((NG, 8, DH), F32)] * 8,
            pltpu.VMEM((8, D), F32), pltpu.VMEM((8, T), F32),
            io, io,
            pltpu.SMEM((TAB_SIZE,), jnp.int32),
            pltpu.SemaphoreType.DMA((NT,)), pltpu.SemaphoreType.DMA((NT,)),
            pltpu.SemaphoreType.DMA((NSLOT + 1,)), pltpu.SemaphoreType.DMA((3,)),
            pltpu.SemaphoreType.DMA((2,)), pltpu.SemaphoreType.DMA((4,)),
        ],
        compiler_params=pltpu.CompilerParams(vmem_limit_bytes=128 * 1024 * 1024),
    )(A_x, grad_out,
      A_k_cache.reshape(a_view), A_v_cache.reshape(a_view),
      A_wq.reshape(wq_view), A_wo.reshape(wo_view),
      B_k_cache.reshape(b_view), B_v_cache.reshape(b_view),
      B_wq.reshape(wq_view), B_wo.reshape(wo_view))
    out, dx, dka, dva, dwqa, dwoa, dkb, dvb, dwqb, dwob = outs
    return (out, dx,
            dka.reshape(cache_shape), dva.reshape(cache_shape),
            dwqa.reshape(A_wq.shape), dwoa.reshape(A_wo.shape),
            dkb.reshape(cache_shape), dvb.reshape(cache_shape),
            dwqb.reshape(B_wq.shape), dwob.reshape(B_wo.shape))
```
